```python
import jax
import jax.numpy as jnp

def _softmax(x, axis=-1):
    return jax.nn.softmax(x, axis=axis)

def _gelu(x):
    return jax.nn.gelu(x, approximate=True)

def _silu(x):
    return jax.nn.silu(x)

def _sigmoid(x):
    return jax.nn.sigmoid(x)

def _layernorm(x, axis=-1, eps=1e-05):
    m = jnp.mean(x, axis=axis, keepdims=True)
    v = jnp.var(x, axis=axis, keepdims=True)
    return (x - m) / jnp.sqrt(v + eps)

def _scatter_add(tgt, idx, src, axis=0):
    return tgt.at[idx].add(src)

def _segment_sum(src, seg, n):
    return jax.ops.segment_sum(src, seg, n)

class _Rng:

    def __init__(self, key):
        self._k = key

    def _next(self):
        self._k, sub = jax.random.split(self._k)
        return sub

    def normal(self, shape):
        return jax.random.normal(self._next(), shape, dtype=jnp.bfloat16)

    def randint(self, lo, hi, shape):
        return jax.random.randint(self._next(), shape, lo, hi, dtype=jnp.int32)

    def uniform(self, shape, lo=0.0, hi=1.0):
        return jax.random.uniform(self._next(), shape, jnp.bfloat16, lo, hi)

    def permutation(self, n):
        return jax.random.permutation(self._next(), n)
kernel_name = 'adaLN_cond__sliding_block_cached__geglu_ffn__decode'

def setup_inputs():
    _rng = _Rng(jax.random.key(int.from_bytes(__import__("os").urandom(4), "little")))
    _w = lambda a: (lambda t: t.astype(jnp.bfloat16) if jnp.issubdtype(t.dtype, jnp.floating) else t)(jnp.asarray(a))

    def _A_setup():
        B, Sq, D = (1, 1, 640)
        Hq, Hkv, Sk, Dh = (32, 32, 32768, 192)
        assert Hq % Hkv == 0, (Hq, Hkv)
        return {'x': _w((lambda *s: _rng.normal(s) * 0.05)(B, Sq, D)), 'k_cache': _w((lambda *s: _rng.normal(s) * 0.05)(B, Hkv, Sk, Dh)), 'v_cache': _w((lambda *s: _rng.normal(s) * 0.05)(B, Hkv, Sk, Dh)), 'wq': _w((lambda *s: _rng.normal(s) * 0.05)(D, Hq * Dh) * D ** (-0.5)), 'wo': _w((lambda *s: _rng.normal(s) * 0.05)(Hq * Dh, D) * (Hq * Dh) ** (-0.5))}
    _A_in = _A_setup()

    def _B_setup():
        B, S, D, F = (1, 1, 640, 1536)
        return {'x': _w((lambda *s: _rng.normal(s) * 0.05)(B, S, D)), 'w_gate': _w((lambda *s: _rng.normal(s) * 0.05)(D, F)), 'w_up': _w((lambda *s: _rng.normal(s) * 0.05)(D, F)), 'w_down': _w((lambda *s: _rng.normal(s) * 0.05)(F, D))}
    _B_in = _B_setup()
    return {'A_x': _A_in['x'], 'A_k_cache': _A_in['k_cache'], 'A_v_cache': _A_in['v_cache'], 'A_wq': _A_in['wq'], 'A_wo': _A_in['wo'], 'B_x': _B_in['x'], 'B_w_gate': _B_in['w_gate'], 'B_w_up': _B_in['w_up'], 'B_w_down': _B_in['w_down'], 'c': _w((lambda *s: _rng.normal(s) * 0.05)(1, 640)), 'w_mod': _w((lambda *s: _rng.normal(s) * 0.05)(640, 6 * 640) * 640 ** (-0.5))}

def reference(A_x, A_k_cache, A_v_cache, A_wq, A_wo, B_x, B_w_gate, B_w_up, B_w_down, c, w_mod):

    def _A_ref(x, k_cache, v_cache, wq, wo):
        B, Sq, D = x.shape
        Hq, Dh = (32, 192)
        Hkv, Sk = (k_cache.shape[1], k_cache.shape[2])
        W = min(4096, max(256, Sk // 4))
        rep = Hq // Hkv
        q = (lambda x, *d: x.transpose(*d))((x @ wq).reshape(B, Sq, Hq, Dh), 0, 2, 1, 3)
        k = jnp.repeat(k_cache[:, :, Sk - W:, :], rep, axis=1)
        v = jnp.repeat(v_cache[:, :, Sk - W:, :], rep, axis=1)
        scores = jnp.einsum('bhqd,bhkd->bhqk', q, k) * Dh ** (-0.5)
        p = _softmax(scores, axis=-1)
        o = jnp.einsum('bhqk,bhkd->bhqd', p, v)
        return (lambda x, *d: x.transpose(*d))(o, 0, 2, 1, 3).reshape(B, Sq, Hq * Dh) @ wo

    def _B_ref(x, w_gate, w_up, w_down):
        return _gelu(x @ w_gate) * (x @ w_up) @ w_down
    x = A_x
    mod = (_silu(c) @ w_mod).reshape(c.shape[0], 6, 1, -1)
    sa, ca, ga, sb, cb, gb = (mod[:, 0].copy(), mod[:, 1].copy(), mod[:, 2].copy(), mod[:, 3].copy(), mod[:, 4].copy(), mod[:, 5].copy())
    h = _layernorm(x, axis=-1) * (1 + ca) + sa
    x = x + ga * _A_ref(h, A_k_cache, A_v_cache, A_wq, A_wo)
    h = _layernorm(x, axis=-1) * (1 + cb) + sb
    x = x + gb * _B_ref(h, B_w_gate, B_w_up, B_w_down)
    return x
```

```python
import numpy as np
import jax
import jax.numpy as jnp
import jax.experimental.pallas as pl
import jax.experimental.pallas.tpu as pltpu

NH = 32
DH = 192
NSLOT = 3
PV_CHUNK = 512
WD_CHUNKS = (768, 512, 256)

F32 = jnp.float32
BF16 = jnp.bfloat16


def _ln(x):
    m = jnp.mean(x, axis=-1, keepdims=True)
    d = x - m
    v = jnp.mean(d * d, axis=-1, keepdims=True)
    return d * jax.lax.rsqrt(v + 1e-5)


def _kernel(x_hbm, c_hbm, wm_hbm, wq_hbm, wo_hbm, kt_hbm, vt_hbm, wg_hbm, wu_hbm, wd_hbm,
            o_ref,
            x_v, c_v, wm_v, wq_v, wo_v, k_v, v_v, wg_v, wu_v, wd_v, q_v, mod_v, acc_v,
            sem_last):
    D = x_v.shape[1]
    SK = kt_hbm.shape[2]
    W = k_v.shape[2]
    nwd = len(WD_CHUNKS)
    offs = [int(o) for o in np.cumsum((0,) + tuple(WD_CHUNKS))]
    scale = float(DH) ** -0.5

    def wd_copy(i, sem):
        return pltpu.make_async_copy(wd_hbm.at[pl.ds(offs[i], WD_CHUNKS[i])],
                                     wd_v.at[pl.ds(offs[i], WD_CHUNKS[i])], sem)

    def down_part(act, i):
        return jnp.dot(act[:, offs[i]:offs[i + 1]], wd_v[pl.ds(offs[i], WD_CHUNKS[i]), :],
                       preferred_element_type=F32)

    def ffn_scope(sem_f):
        cp_wg = pltpu.make_async_copy(wg_hbm, wg_v, sem_f.at[0])
        cp_wu = pltpu.make_async_copy(wu_hbm, wu_v, sem_f.at[1])
        cp_wd = [wd_copy(i, sem_f.at[2 + i]) for i in range(nwd - 1)]
        cp_wd.append(wd_copy(nwd - 1, sem_last))

        def attn_scope(sem_k, sem_v):
            def cp_k(h, slot):
                return pltpu.make_async_copy(kt_hbm.at[h, :, pl.ds(SK - W, W)], k_v.at[slot],
                                             sem_k.at[slot])

            def cp_v(h, slot):
                return pltpu.make_async_copy(vt_hbm.at[h, :, pl.ds(SK - W, W)], v_v.at[slot],
                                             sem_v.at[slot])

            def prologue(sem_p):
                cp_c = pltpu.make_async_copy(c_hbm, c_v, sem_p.at[0])
                cp_x = pltpu.make_async_copy(x_hbm, x_v, sem_p.at[1])
                cp_wm = pltpu.make_async_copy(wm_hbm, wm_v, sem_p.at[2])
                cp_wq = pltpu.make_async_copy(wq_hbm, wq_v, sem_p.at[3])
                cp_wo = pltpu.make_async_copy(wo_hbm, wo_v, sem_p.at[4])
                cp_c.start()
                cp_x.start()
                cp_wm.start()
                cp_wq.start()
                cp_wo.start()
                for j in range(NSLOT):
                    cp_k(j, j).start(priority=0)
                    cp_v(j, j).start(priority=1)
                acc_v[...] = jnp.zeros(acc_v.shape, F32)

                cp_c.wait()
                cc = c_v[...].astype(F32)
                sc = (cc * jax.nn.sigmoid(cc)).astype(BF16)
                cp_wm.wait()
                mod = jnp.dot(sc, wm_v[...], preferred_element_type=F32).astype(BF16).astype(F32)
                for j in range(6):
                    mod_v[j] = mod[:, j * D:(j + 1) * D]
                cp_x.wait()
                x = x_v[...].astype(F32)
                h1 = (_ln(x) * (1.0 + mod_v[1]) + mod_v[0]).astype(BF16)

                cp_wq.wait()
                q = jnp.dot(h1, wq_v[...], preferred_element_type=F32).astype(BF16)
                for hh in range(NH):
                    q_v[hh] = q[:, hh * DH:(hh + 1) * DH]
                cp_wo.wait()

            pl.run_scoped(prologue, pltpu.SemaphoreType.DMA((5,)))

            def head(h, carry):
                slot = h % NSLOT
                cp_k(h, slot).wait()
                s = jnp.dot(q_v[h], k_v[slot], preferred_element_type=F32) * scale
                m = jnp.max(s, axis=-1, keepdims=True)
                p = jnp.exp(s - m)
                l = jnp.sum(p, axis=-1, keepdims=True)
                cp_v(h, slot).wait()
                acc = None
                for j in range(W // PV_CHUNK):
                    vt = v_v[slot, :, pl.ds(j * PV_CHUNK, PV_CHUNK)].astype(F32)
                    prod = vt * p[:, j * PV_CHUNK:(j + 1) * PV_CHUNK]
                    for t in range(PV_CHUNK // 128):
                        piece = prod[:, t * 128:(t + 1) * 128]
                        acc = piece if acc is None else acc + piece
                o_col = jnp.sum(acc, axis=-1, keepdims=True) / l
                o_col = o_col.astype(BF16).astype(F32)

                @pl.when(h + NSLOT < NH)
                def _():
                    cp_k(h + NSLOT, slot).start(priority=0)
                    cp_v(h + NSLOT, slot).start(priority=1)

                @pl.when(h + NSLOT == NH)
                def _():
                    cp_wg.start(priority=1)

                @pl.when(h + NSLOT == NH + 1)
                def _():
                    cp_wu.start(priority=1)

                @pl.when(h + NSLOT == NH + 2)
                def _():
                    for cp in cp_wd:
                        cp.start(priority=1)

                wo_h = wo_v[pl.ds(pl.multiple_of(h * DH, 16), DH), :].astype(F32)
                acc_v[...] += (o_col * wo_h).reshape(DH // 8, 8, D).sum(axis=0)
                return carry

            jax.lax.fori_loop(0, NH, head, 0)

        pl.run_scoped(attn_scope, pltpu.SemaphoreType.DMA((NSLOT,)),
                      pltpu.SemaphoreType.DMA((NSLOT,)))

        attn = jnp.sum(acc_v[...], axis=0, keepdims=True)
        x1 = x_v[...].astype(F32) + mod_v[2] * attn
        h2 = (_ln(x1) * (1.0 + mod_v[4]) + mod_v[3]).astype(BF16)
        cp_wg.wait()
        g = jnp.dot(h2, wg_v[...], preferred_element_type=F32)
        cp_wu.wait()
        u = jnp.dot(h2, wu_v[...], preferred_element_type=F32)
        act = (jax.nn.gelu(g, approximate=True) * u).astype(BF16)
        ffn = None
        for i in range(nwd - 1):
            cp_wd[i].wait()
            part = down_part(act, i)
            ffn = part if ffn is None else ffn + part
        return x1, act, ffn

    x1, act, ffn = pl.run_scoped(ffn_scope, pltpu.SemaphoreType.DMA((nwd + 1,)))
    wd_copy(nwd - 1, sem_last).wait()
    o_ref[...] = (x1 + mod_v[5] * (ffn + down_part(act, nwd - 1))).astype(o_ref.dtype)


@jax.jit
def pallas_adaLN_cond__sliding_block_cached__geglu_ffn__decode_kernel(
    A_x: jax.Array,
    A_k_cache: jax.Array,
    A_v_cache: jax.Array,
    A_wq: jax.Array,
    A_wo: jax.Array,
    B_x: jax.Array,
    B_w_gate: jax.Array,
    B_w_up: jax.Array,
    B_w_down: jax.Array,
    c: jax.Array,
    w_mod: jax.Array,
):
    del B_x
    B, Sq, D = A_x.shape
    _, Hkv, SK, Dh = A_k_cache.shape
    assert B == 1 and Sq == 1 and Hkv == NH and Dh == DH
    assert B_w_down.shape[0] == sum(WD_CHUNKS)
    W = min(4096, max(256, SK // 4))
    kt = jnp.swapaxes(A_k_cache, 2, 3).reshape(Hkv, Dh, SK)
    vt = jnp.swapaxes(A_v_cache, 2, 3).reshape(Hkv, Dh, SK)
    any_spec = pl.BlockSpec(memory_space=pl.ANY)
    out = pl.pallas_call(
        _kernel,
        in_specs=[any_spec] * 10,
        out_specs=pl.BlockSpec(memory_space=pltpu.VMEM),
        out_shape=jax.ShapeDtypeStruct((1, D), A_x.dtype),
        scratch_shapes=[
            pltpu.VMEM((1, D), BF16), pltpu.VMEM((1, D), BF16),
            pltpu.VMEM(w_mod.shape, BF16), pltpu.VMEM(A_wq.shape, BF16),
            pltpu.VMEM(A_wo.shape, BF16),
            pltpu.VMEM((NSLOT, Dh, W), BF16), pltpu.VMEM((NSLOT, Dh, W), BF16),
            pltpu.VMEM(B_w_gate.shape, BF16), pltpu.VMEM(B_w_up.shape, BF16),
            pltpu.VMEM(B_w_down.shape, BF16),
            pltpu.VMEM((NH, 1, Dh), BF16), pltpu.VMEM((6, 1, D), F32), pltpu.VMEM((8, D), F32),
            pltpu.SemaphoreType.DMA,
        ],
        compiler_params=pltpu.CompilerParams(vmem_limit_bytes=100 * 1024 * 1024),
    )(A_x.reshape(1, D), c, w_mod, A_wq, A_wo, kt, vt, B_w_gate, B_w_up, B_w_down)
    return out.reshape(B, Sq, D)
```

```python
import contextlib
import functools
import numpy as np
import jax
import jax.numpy as jnp
from jax import lax
from jax.experimental import pallas as pl
from jax.experimental.pallas import tpu as pltpu

NH, DH = 32, 192
NG = DH // 8
F32 = jnp.float32
BF16 = jnp.bfloat16


def _ln(x):
    m = jnp.mean(x, axis=-1, keepdims=True)
    d = x - m
    v = jnp.mean(d * d, axis=-1, keepdims=True)
    return d * jax.lax.rsqrt(v + 1e-5)


def _tree_sum(xs):
    xs = list(xs)
    while len(xs) > 1:
        nxt = [xs[i] + xs[i + 1] for i in range(0, len(xs) - 1, 2)]
        if len(xs) % 2:
            nxt.append(xs[-1])
        xs = nxt
    return xs[0]


def make(scopes=False, wd_chunks=(768, 512, 256), win=32, nobc=True, nosc=False, PC=1024, KPAD=256,
         nbm=10, nbq=24, qblk=4, overlap=True, nbt=17, mblk=6):
    def scope(name):
        return jax.named_scope(name) if scopes else contextlib.nullcontext()

    def kernel(x_hbm, c_hbm, wm_hbm, wq_hbm, wo_hbm, kt_hbm, vt_hbm, wg_hbm, wu_hbm, wd_hbm,
               o_ref,
               x_v, c_v, wm_v, wq_v, wo_v, k_v, v_v, wg_v, wu_v, wd_v, qb_v, s_v, po_v, mod_v, acc_v,
               sem_last):
        D = x_v.shape[1]
        SK = kt_hbm.shape[2]
        W = v_v.shape[2]
        nwd = len(wd_chunks)
        offs = [int(o) for o in np.cumsum((0,) + tuple(wd_chunks))]
        scale = float(DH) ** -0.5 * float(np.log2(np.e))
        CS = W // PC
        P = NG * CS
        SH = int(np.log2(CS))
        NT = W // 128
        NA = NT
        assert P % win == 0 and win == NA
        NC2 = P - NA - 2 * NG

        def wd_copy(i, sem):
            return pltpu.make_async_copy(wd_hbm.at[pl.ds(offs[i], wd_chunks[i])],
                                         wd_v.at[pl.ds(offs[i], wd_chunks[i])], sem)

        def down_part(act, i):
            return jnp.dot(act[:, offs[i]:offs[i + 1]], wd_v[pl.ds(offs[i], wd_chunks[i]), :],
                           preferred_element_type=F32)

        def ffn_scope(sem_f):
            cp_wg = pltpu.make_async_copy(wg_hbm, wg_v, sem_f.at[0])
            cp_wu = pltpu.make_async_copy(wu_hbm, wu_v, sem_f.at[1])
            cp_wd = [wd_copy(i, sem_f.at[2 + i]) for i in range(nwd - 1)] + [wd_copy(nwd - 1, sem_last)]

            def attn_scope(sem_k, sem_v):
                def gc(j):
                    return j >> SH, pl.multiple_of((j & (CS - 1)) * PC, PC)

                def vstart(h, slot, j, sj):
                    g, c = gc(j)
                    pltpu.make_async_copy(vt_hbm.at[h * NG + g, :, pl.ds(SK - W + c, PC)],
                                          v_v.at[slot * NG + g, :, pl.ds(c, PC)], sem_v.at[sj & (win - 1)]).start(priority=1)

                def wait16(j):
                    d = v_v.at[0, :, pl.ds(0, PC)]
                    pltpu.make_async_copy(d, d, sem_v.at[j & (win - 1)]).wait()

                def kstart(h, slot, j):
                    g, c = gc(j)
                    pltpu.make_async_copy(kt_hbm.at[h * NG + g, :, pl.ds(SK - W + c, PC)],
                                          k_v.at[slot * NG + g, :, pl.ds(c, PC)], sem_k.at[slot]).start(priority=0)

                def kwait_all(slot):
                    d = k_v.at[pl.ds(slot * NG, NG), :, pl.ds(0, W)]
                    pltpu.make_async_copy(d, d, sem_k.at[slot]).wait()

                def prologue(sem_p):
                    cp_c = pltpu.make_async_copy(c_hbm, c_v, sem_p.at[0])
                    cp_x = pltpu.make_async_copy(x_hbm, x_v, sem_p.at[1])
                    cp_c.start()
                    cp_x.start()
                    NQ = 6
                    QC = wq_v.shape[1] // NQ
                    MC = wm_v.shape[1] // NQ
                    B1 = (D // 8) * NQ
                    NW1 = 256
                    NWO = NH * NG // 2
                    B2 = B1 + 2 * P
                    B3 = B1 + NW1
                    B4 = B3 + P
                    B5 = B2 + (NWO - NW1)
                    assert B2 <= B3 <= B5 - win and B5 <= B4 and B4 % win == 0 and B1 % win == 0 and B3 % win == 0

                    def t1_wq(b):
                        g = lax.div(b, NQ)
                        r = pl.multiple_of(g * 8, 8)
                        cq = pl.multiple_of((b - g * NQ) * QC, 128)
                        pltpu.make_async_copy(wq_hbm.at[pl.ds(r, 8), pl.ds(cq, QC)],
                                              wq_v.at[pl.ds(r, 8), pl.ds(cq, QC)], sem_v.at[b & (win - 1)]).start(priority=1)

                    def t0_wm(b):
                        g = lax.div(b, NQ)
                        r = pl.multiple_of(g * 8, 8)
                        cm = pl.multiple_of((b - g * NQ) * MC, 128)
                        pltpu.make_async_copy(wm_hbm.at[pl.ds(r, 8), pl.ds(cm, MC)],
                                              wm_v.at[pl.ds(r, 8), pl.ds(cm, MC)], sem_p.at[2]).start(priority=0)

                    def wo_copy(i, sem):
                        return pltpu.make_async_copy(wo_hbm.at[pl.ds(2 * i, 2)], wo_v.at[pl.ds(2 * i, 2)], sem)

                    def wait_wo(b):
                        wo_copy(0, sem_v.at[b & (win - 1)]).wait()

                    def beats(lo, n, wait, t1, t0):
                        def body(i, carry):
                            b = lo + i
                            if wait is not None:
                                wait(b)
                            t1(b)
                            if t0 is not None:
                                t0(b)
                            return carry
                        if n > 0:
                            lax.fori_loop(0, n, body, 0)

                    t1_wo = lambda b: wo_copy(b - B1, sem_v.at[b & (win - 1)]).start(priority=1)
                    t1_v0 = lambda b: vstart(0, 0, b - B3, b)

                    def t0_k(b):
                        m = b - B1
                        hh = (m >= P).astype(jnp.int32)
                        kstart(hh, hh, m - hh * P)
                    t0_wo = lambda b: wo_copy(b - B2 + NW1, sem_p.at[3]).start(priority=0)

                    segs = [(0, None, t1_wq, t0_wm), (win, wait16, t1_wq, t0_wm),
                            (B1, wait16, t1_wo, t0_k), (B1 + win, wait_wo, t1_wo, t0_k),
                            (B2, wait_wo, t1_wo, t0_wo), (B3, wait_wo, t1_v0, t0_wo),
                            (B3 + win, wait16, t1_v0, t0_wo), (B5, wait16, t1_v0, None), (B4, None, None, None)]
                    cur = [0]

                    def emit(n):
                        lo, hi = cur[0], min(cur[0] + n, B4)
                        for (a, wait, t1, t0), nxt in zip(segs[:-1], segs[1:]):
                            s0, s1 = max(lo, a), min(hi, nxt[0])
                            if s1 > s0:
                                beats(s0, s1 - s0, wait, t1, t0)
                        cur[0] = hi

                    with scope("s1"):
                        emit(B1 + win)
                    acc_v[...] = jnp.zeros(acc_v.shape, F32)
                    with scope("mod"):
                        cp_c.wait()
                        cc = c_v[...].astype(F32)
                        sc = (cc * jax.nn.sigmoid(cc)).astype(BF16)
                        pltpu.make_async_copy(wm_v, wm_v, sem_p.at[2]).wait()
                        mpb = 6 // mblk
                        for j in range(mblk):
                            w = wm_v[:, pl.ds(j * mpb * D, mpb * D)]
                            md = jnp.dot(sc, w, preferred_element_type=F32).astype(BF16).astype(F32)
                            for u in range(mpb):
                                mod_v[j * mpb + u] = md[:, u * D:(u + 1) * D]
                            emit(nbm)
                        cp_x.wait()
                        x = x_v[...].astype(F32)
                        h1 = (_ln(x) * (1.0 + mod_v[1]) + mod_v[0]).astype(BF16)
                    with scope("qproj"):
                        QB = NH * DH // qblk

                        def q_mm(j):
                            w = wq_v[:, pl.ds(j * QB, QB)]
                            return jnp.dot(h1, w, preferred_element_type=F32).astype(BF16).astype(F32) * scale

                        def q_tr(j, q):
                            for u in range(QB // 128):
                                row = q[:, u * 128:(u + 1) * 128]
                                qb_v[pl.ds(j * QB + u * 128, 128), :] = jnp.broadcast_to(row, (128, 128)).T
                        if overlap:
                            q = q_mm(0)
                            emit(nbt)
                            for j in range(qblk):
                                qn = q_mm(j + 1) if j + 1 < qblk else None
                                q_tr(j, q)
                                emit(nbq if j + 1 < qblk else nbt)
                                q = qn
                        else:
                            for j in range(qblk):
                                q = q_mm(j)
                                emit(nbt)
                                q_tr(j, q)
                                emit(nbt)
                    with scope("s2"):
                        emit(B4)
                        d = wo_v.at[pl.ds(2 * NW1, NH * NG - 2 * NW1)]
                        pltpu.make_async_copy(d, d, sem_p.at[3]).wait()

                pl.run_scoped(prologue, pltpu.SemaphoreType.DMA((4,)))

                def head(h, kslot, do_k, do_v):
                    k_in = jnp.where(kslot == 0, 2, kslot - 1)
                    vslot = h & 1
                    v_in = 1 - vslot

                    def beat(j):
                        if do_v:
                            vstart(h + 1, v_in, j, j)
                        if do_k:
                            kstart(h + 2, k_in, j)

                    with scope("kwait"):
                        kwait_all(kslot)

                    with scope("qk"):
                        qb = qb_v[pl.ds(pl.multiple_of(h * DH, 8), DH), :]
                        qb = [qb[8 * g:8 * g + 8] for g in range(NG)]

                        def loop_a(t, mx):
                            wait16(t)
                            off = pl.multiple_of(t * 128, 128)
                            kt = k_v[pl.ds(kslot * NG, NG), :, pl.ds(off, 128)].astype(F32)
                            part = _tree_sum([kt[g] * qb[g] for g in range(NG)])
                            s = jnp.broadcast_to(jnp.sum(part, axis=0, keepdims=True), (8, 128))
                            s_v[:, pl.ds(off, 128)] = s
                            beat(t)
                            return jnp.maximum(mx, s)
                        mx = lax.fori_loop(0, NA, loop_a, jnp.full((8, 128), -jnp.inf, F32))
                        m = jnp.max(mx, axis=1, keepdims=True)

                    with scope("mid"):
                        p = jnp.exp2(s_v[...] - m)
                        l = _tree_sum([p[:, t * 128:(t + 1) * 128] for t in range(NT)])
                        inv_l = 1.0 / jnp.sum(l, axis=1, keepdims=True)

                    with scope("pv"):
                        def loop_b(g, carry):
                            if do_v:
                                wait16(g + NA)
                            vt = v_v[vslot * NG + g].astype(F32)
                            prod = vt * p
                            po_v[g] = _tree_sum([prod[:, t * 128:(t + 1) * 128] for t in range(NT)])
                            beat(g + NA)
                            return carry
                        lax.fori_loop(0, NG, loop_b, 0)

                    with scope("ored"):
                        for g in range(NG):
                            o8 = jnp.sum(po_v[g], axis=1, keepdims=True) * inv_l
                            po_v[g] = jnp.broadcast_to(o8.astype(BF16).astype(F32), (8, 128))

                    with scope("wo"):
                        def loop_c(g, acc):
                            if do_v:
                                wait16(g + NA + NG)
                            w = wo_v[h * NG + g].astype(F32)
                            new = acc + jnp.concatenate([po_v[g]] * (D // 128), axis=1) * w
                            beat(g + NA + NG)
                            return new
                        acc = lax.fori_loop(0, NG, loop_c, jnp.zeros((8, D), F32))
                        acc_v[...] += acc

                    if do_v:
                        with scope("idle"):
                            def loop_d(t, carry):
                                wait16(t + NA + 2 * NG)
                                beat(t + NA + 2 * NG)
                                return carry
                            lax.fori_loop(0, NC2, loop_d, 0)
                    return jnp.where(kslot == 2, 0, kslot + 1)

                kslot = lax.fori_loop(0, NH - 2, lambda h, ks: head(h, ks, True, True), jnp.int32(0))
                kslot = head(jnp.int32(NH - 2), kslot, False, True)
                cp_wg.start(priority=1)
                cp_wu.start(priority=1)
                for cp in cp_wd:
                    cp.start(priority=1)
                head(jnp.int32(NH - 1), kslot, False, False)

            pl.run_scoped(attn_scope, pltpu.SemaphoreType.DMA((3,)), pltpu.SemaphoreType.DMA((win,)))

            with scope("post"):
                attn = jnp.sum(acc_v[...], axis=0, keepdims=True)
                x1 = x_v[...].astype(F32) + mod_v[2] * attn
                h2 = (_ln(x1) * (1.0 + mod_v[4]) + mod_v[3]).astype(BF16)
            with scope("gate"):
                cp_wg.wait()
                g = jnp.dot(h2, wg_v[...], preferred_element_type=F32)
            with scope("up"):
                cp_wu.wait()
                u = jnp.dot(h2, wu_v[...], preferred_element_type=F32)
                act = (jax.nn.gelu(g, approximate=True) * u).astype(BF16)
            ffn = None
            for i in range(nwd - 1):
                with scope(f"down{i}"):
                    cp_wd[i].wait()
                    part = down_part(act, i)
                    ffn = part if ffn is None else ffn + part
            return x1, act, ffn

        x1, act, ffn = pl.run_scoped(ffn_scope, pltpu.SemaphoreType.DMA((nwd + 1,)))
        with scope("downlast"):
            wd_copy(nwd - 1, sem_last).wait()
            o_ref[...] = (x1 + mod_v[5] * (ffn + down_part(act, nwd - 1))).astype(o_ref.dtype)

    def fn(A_x, A_k_cache, A_v_cache, A_wq, A_wo, B_x, B_w_gate, B_w_up, B_w_down, c, w_mod):
        B, Sq, D = A_x.shape
        _, Hkv, SK, Dh = A_k_cache.shape
        assert B == 1 and Sq == 1 and Hkv == NH and Dh == DH
        W = min(4096, max(256, SK // 4))
        kt = jnp.swapaxes(A_k_cache, 2, 3).reshape(Hkv * NG, 8, SK)
        vt = jnp.swapaxes(A_v_cache, 2, 3).reshape(Hkv * NG, 8, SK)
        x2 = A_x.reshape(1, D)
        any_spec = pl.BlockSpec(memory_space=pl.ANY)
        out = pl.pallas_call(
            kernel,
            in_specs=[any_spec] * 10,
            out_specs=pl.BlockSpec(memory_space=pltpu.VMEM),
            out_shape=jax.ShapeDtypeStruct((1, D), A_x.dtype),
            scratch_shapes=[
                pltpu.VMEM((1, D), BF16), pltpu.VMEM((1, D), BF16),
                pltpu.VMEM(w_mod.shape, BF16), pltpu.VMEM(A_wq.shape, BF16), pltpu.VMEM((NH * NG, 8, D), BF16),
                pltpu.VMEM((3 * NG, 8, W + KPAD), BF16), pltpu.VMEM((2 * NG, 8, W), BF16),
                pltpu.VMEM(B_w_gate.shape, BF16), pltpu.VMEM(B_w_up.shape, BF16), pltpu.VMEM(B_w_down.shape, BF16),
                pltpu.VMEM((NH * Dh, 128), F32), pltpu.VMEM((8, W), F32),
                pltpu.VMEM((NG, 8, 128), F32),
                pltpu.VMEM((6, 1, D), F32), pltpu.VMEM((8, D), F32),
                pltpu.SemaphoreType.DMA,
            ],
            compiler_params=pltpu.CompilerParams(vmem_limit_bytes=100 * 1024 * 1024, disable_bounds_checks=nobc,
                                                 disable_semaphore_checks=nosc),
        )(x2, c, w_mod, A_wq, A_wo.reshape(NH * NG, 8, D), kt, vt, B_w_gate, B_w_up, B_w_down)
        return out.reshape(B, Sq, D)
    return fn


_impl = make()


@jax.jit
def pallas_adaLN_cond__sliding_block_cached__geglu_ffn__decode_kernel(
    A_x: jax.Array,
    A_k_cache: jax.Array,
    A_v_cache: jax.Array,
    A_wq: jax.Array,
    A_wo: jax.Array,
    B_x: jax.Array,
    B_w_gate: jax.Array,
    B_w_up: jax.Array,
    B_w_down: jax.Array,
    c: jax.Array,
    w_mod: jax.Array,
):
    return _impl(A_x, A_k_cache, A_v_cache, A_wq, A_wo, B_x, B_w_gate, B_w_up, B_w_down, c, w_mod)
```

```python
import contextlib
import functools
import numpy as np
import jax
import jax.numpy as jnp
from jax import lax
from jax.experimental import pallas as pl
from jax.experimental.pallas import tpu as pltpu

NH, DH = 32, 192
NG = DH // 8
F32 = jnp.float32
BF16 = jnp.bfloat16


def _ln(x):
    m = jnp.mean(x, axis=-1, keepdims=True)
    d = x - m
    v = jnp.mean(d * d, axis=-1, keepdims=True)
    return d * jax.lax.rsqrt(v + 1e-5)


def _tree_sum(xs):
    xs = list(xs)
    while len(xs) > 1:
        nxt = [xs[i] + xs[i + 1] for i in range(0, len(xs) - 1, 2)]
        if len(xs) % 2:
            nxt.append(xs[-1])
        xs = nxt
    return xs[0]


def make(scopes=False, wd_chunks=(768, 512, 256), win=32, nobc=True, nosc=False, PC=512, GP=3, order='c', KPAD=256,
         nbm=12, nbq=20, qblk=4, overlap=True, nbt=14, mblk=6, nw1=224):
    def scope(name):
        return jax.named_scope(name) if scopes else contextlib.nullcontext()

    def kernel(x_hbm, c_hbm, wm_hbm, wq_hbm, wo_hbm, kt_hbm, vt_hbm, wg_hbm, wu_hbm, wd_hbm,
               o_ref,
               x_v, c_v, wm_v, wq_v, wo_v, k_v, v_v, wg_v, wu_v, wd_v, qb_v, s_v, po_v, mod_v, acc_v,
               sem_last):
        D = x_v.shape[1]
        SK = kt_hbm.shape[2]
        W = v_v.shape[2]
        nwd = len(wd_chunks)
        offs = [int(o) for o in np.cumsum((0,) + tuple(wd_chunks))]
        scale = float(DH) ** -0.5 * float(np.log2(np.e))
        CS = W // PC
        RS = NG // GP
        P = RS * CS
        NT = W // 128
        NA = NT
        assert P % win == 0 and win == NA
        NC = P - NA - NG
        NC1 = min(NC, NG)
        GC = NG // NC1
        NC2 = NC - NC1
        assert NC1 * GC == NG

        def wd_copy(i, sem):
            return pltpu.make_async_copy(wd_hbm.at[pl.ds(offs[i], wd_chunks[i])],
                                         wd_v.at[pl.ds(offs[i], wd_chunks[i])], sem)

        def down_part(act, i):
            return jnp.dot(act[:, offs[i]:offs[i + 1]], wd_v[pl.ds(offs[i], wd_chunks[i]), :],
                           preferred_element_type=F32)

        def ffn_scope(sem_f):
            cp_wg = pltpu.make_async_copy(wg_hbm, wg_v, sem_f.at[0])
            cp_wu = pltpu.make_async_copy(wu_hbm, wu_v, sem_f.at[1])
            cp_wd = [wd_copy(i, sem_f.at[2 + i]) for i in range(nwd - 1)] + [wd_copy(nwd - 1, sem_last)]

            def attn_scope(sem_k, sem_v):
                def gc(j):
                    if order == 'r':
                        a = j >> int(np.log2(CS))
                        b = j & (CS - 1)
                    elif RS & (RS - 1) == 0:
                        b = j >> int(np.log2(RS))
                        a = j & (RS - 1)
                    else:
                        b = lax.div(j, RS)
                        a = j - b * RS
                    return a * GP, pl.multiple_of(b * PC, PC)

                def vstart(h, slot, j, sj):
                    g, c = gc(j)
                    pltpu.make_async_copy(vt_hbm.at[pl.ds(h * NG + g, GP), :, pl.ds(SK - W + c, PC)],
                                          v_v.at[pl.ds(slot * NG + g, GP), :, pl.ds(c, PC)],
                                          sem_v.at[sj & (win - 1)]).start(priority=1)

                def waitv(j):
                    d = v_v.at[pl.ds(0, GP), :, pl.ds(0, PC)]
                    pltpu.make_async_copy(d, d, sem_v.at[j & (win - 1)]).wait()

                def kstart(h, slot, j):
                    g, c = gc(j)
                    pltpu.make_async_copy(kt_hbm.at[pl.ds(h * NG + g, GP), :, pl.ds(SK - W + c, PC)],
                                          k_v.at[pl.ds(slot * NG + g, GP), :, pl.ds(c, PC)],
                                          sem_k.at[slot]).start(priority=0)

                def kwait_all(slot):
                    d = k_v.at[pl.ds(slot * NG, NG), :, pl.ds(0, W)]
                    pltpu.make_async_copy(d, d, sem_k.at[slot]).wait()

                def prologue(sem_p):
                    cp_c = pltpu.make_async_copy(c_hbm, c_v, sem_p.at[0])
                    cp_x = pltpu.make_async_copy(x_hbm, x_v, sem_p.at[1])
                    cp_c.start()
                    cp_x.start()
                    NQ = 6
                    QC = wq_v.shape[1] // NQ
                    MC = wm_v.shape[1] // NQ
                    B1 = (D // 8) * NQ
                    NW1 = nw1
                    NWO = NH * NG // 2
                    B2 = B1 + (NWO - NW1)
                    B3 = B1 + NW1
                    B4 = B3 + P
                    B5 = B2 + 2 * P
                    assert B5 <= B4 and B4 % win == 0 and B1 % win == 0 and B3 % win == 0

                    def t1_wq(b):
                        g = lax.div(b, NQ)
                        r = pl.multiple_of(g * 8, 8)
                        cq = pl.multiple_of((b - g * NQ) * QC, 128)
                        pltpu.make_async_copy(wq_hbm.at[pl.ds(r, 8), pl.ds(cq, QC)],
                                              wq_v.at[pl.ds(r, 8), pl.ds(cq, QC)], sem_v.at[b & (win - 1)]).start(priority=1)

                    def t0_wm(b):
                        g = lax.div(b, NQ)
                        r = pl.multiple_of(g * 8, 8)
                        cm = pl.multiple_of((b - g * NQ) * MC, 128)
                        pltpu.make_async_copy(wm_hbm.at[pl.ds(r, 8), pl.ds(cm, MC)],
                                              wm_v.at[pl.ds(r, 8), pl.ds(cm, MC)], sem_p.at[2]).start(priority=0)

                    def wo_copy(i, sem):
                        return pltpu.make_async_copy(wo_hbm.at[pl.ds(2 * i, 2)], wo_v.at[pl.ds(2 * i, 2)], sem)

                    def wait16(b):
                        d = wq_v.at[pl.ds(0, 8), pl.ds(0, QC)]
                        pltpu.make_async_copy(d, d, sem_v.at[b & (win - 1)]).wait()

                    def wait_wo(b):
                        wo_copy(0, sem_v.at[b & (win - 1)]).wait()

                    def beats(lo, n, wait, t1, t0):
                        def body(i, carry):
                            b = lo + i
                            if wait is not None:
                                wait(b)
                            t1(b)
                            if t0 is not None:
                                t0(b)
                            return carry
                        if n > 0:
                            lax.fori_loop(0, n, body, 0)

                    t1_wo = lambda b: wo_copy(b - B1, sem_v.at[b & (win - 1)]).start(priority=1)
                    t1_v0 = lambda b: vstart(0, 0, b - B3, b)

                    def t0_k(b):
                        m = b - B2
                        hh = (m >= P).astype(jnp.int32)
                        kstart(hh, hh, m - hh * P)
                    t0_wo = lambda b: wo_copy(b - B1 + NW1, sem_p.at[3]).start(priority=0)

                    def pick(b, table):
                        for lo_, f_ in table[::-1]:
                            if b >= lo_:
                                return f_
                    tw = [(0, None), (win, wait16), (B1 + win, wait_wo), (B3 + win, waitv)]
                    t1t = [(0, t1_wq), (B1, t1_wo), (B3, t1_v0)]
                    t0t = [(0, t0_wm), (B1, t0_wo), (B2, t0_k), (B5, None)]
                    cuts = sorted(set([x[0] for x in tw + t1t + t0t if x[0] < B4] + [B4]))
                    segs = [(a, pick(a, tw), pick(a, t1t), pick(a, t0t)) for a in cuts]
                    cur = [0]

                    def emit(n):
                        lo, hi = cur[0], min(cur[0] + n, B4)
                        for (a, wait, t1, t0), nxt in zip(segs[:-1], segs[1:]):
                            s0, s1 = max(lo, a), min(hi, nxt[0])
                            if s1 > s0:
                                beats(s0, s1 - s0, wait, t1, t0)
                        cur[0] = hi

                    with scope("s1"):
                        emit(B1 + win)
                    acc_v[...] = jnp.zeros(acc_v.shape, F32)
                    with scope("mod"):
                        cp_c.wait()
                        cc = c_v[...].astype(F32)
                        sc = (cc * jax.nn.sigmoid(cc)).astype(BF16)
                        pltpu.make_async_copy(wm_v, wm_v, sem_p.at[2]).wait()
                        mpb = 6 // mblk
                        for j in range(mblk):
                            w = wm_v[:, pl.ds(j * mpb * D, mpb * D)]
                            md = jnp.dot(sc, w, preferred_element_type=F32).astype(BF16).astype(F32)
                            for u in range(mpb):
                                mod_v[j * mpb + u] = md[:, u * D:(u + 1) * D]
                            emit(nbm)
                        cp_x.wait()
                        x = x_v[...].astype(F32)
                        h1 = (_ln(x) * (1.0 + mod_v[1]) + mod_v[0]).astype(BF16)
                    with scope("qproj"):
                        QB = NH * DH // qblk

                        def q_mm(j):
                            w = wq_v[:, pl.ds(j * QB, QB)]
                            return jnp.dot(h1, w, preferred_element_type=F32).astype(BF16).astype(F32) * scale

                        def q_tr(j, q):
                            for u in range(QB // 128):
                                row = q[:, u * 128:(u + 1) * 128]
                                qb_v[pl.ds(j * QB + u * 128, 128), :] = jnp.broadcast_to(row, (128, 128)).T
                        if overlap:
                            q = q_mm(0)
                            emit(nbt)
                            for j in range(qblk):
                                qn = q_mm(j + 1) if j + 1 < qblk else None
                                q_tr(j, q)
                                emit(nbq if j + 1 < qblk else nbt)
                                q = qn
                        else:
                            for j in range(qblk):
                                q = q_mm(j)
                                emit(nbt)
                                q_tr(j, q)
                                emit(nbt)
                    with scope("s2"):
                        emit(B4)
                        d = wo_v.at[pl.ds(2 * NW1, NH * NG - 2 * NW1)]
                        pltpu.make_async_copy(d, d, sem_p.at[3]).wait()

                pl.run_scoped(prologue, pltpu.SemaphoreType.DMA((4,)))

                def head(h, kslot, do_k, do_v):
                    k_in = jnp.where(kslot == 0, 2, kslot - 1)
                    vslot = h & 1
                    v_in = 1 - vslot

                    def beat(j):
                        if do_v:
                            vstart(h + 1, v_in, j, j)
                        if do_k:
                            kstart(h + 2, k_in, j)

                    with scope("kwait"):
                        kwait_all(kslot)

                    with scope("qk"):
                        qb = qb_v[pl.ds(pl.multiple_of(h * DH, 8), DH), :]
                        qb = [qb[8 * g:8 * g + 8] for g in range(NG)]

                        def loop_a(t, mx):
                            waitv(t)
                            off = pl.multiple_of(t * 128, 128)
                            kt = k_v[pl.ds(kslot * NG, NG), :, pl.ds(off, 128)].astype(F32)
                            part = _tree_sum([kt[g] * qb[g] for g in range(NG)])
                            s = jnp.broadcast_to(jnp.sum(part, axis=0, keepdims=True), (8, 128))
                            s_v[:, pl.ds(off, 128)] = s
                            beat(t)
                            return jnp.maximum(mx, s)
                        mx = lax.fori_loop(0, NA, loop_a, jnp.full((8, 128), -jnp.inf, F32))
                        m = jnp.max(mx, axis=1, keepdims=True)

                    with scope("mid"):
                        p = jnp.exp2(s_v[...] - m)
                        l = _tree_sum([p[:, t * 128:(t + 1) * 128] for t in range(NT)])
                        inv_l = 1.0 / jnp.sum(l, axis=1, keepdims=True)

                    with scope("pv"):
                        def loop_b(g, carry):
                            if do_v:
                                waitv(g + NA)
                            vt = v_v[vslot * NG + g].astype(F32)
                            prod = vt * p
                            po_v[g] = _tree_sum([prod[:, t * 128:(t + 1) * 128] for t in range(NT)])
                            beat(g + NA)
                            return carry
                        lax.fori_loop(0, NG, loop_b, 0)

                    with scope("ored"):
                        for g in range(NG):
                            o8 = jnp.sum(po_v[g], axis=1, keepdims=True) * inv_l
                            po_v[g] = jnp.broadcast_to(o8.astype(BF16).astype(F32), (8, 128))

                    with scope("wo"):
                        def loop_c(i, acc):
                            if do_v:
                                waitv(i + NA + NG)
                            for u in range(GC):
                                g = i * GC + u
                                w = wo_v[h * NG + g].astype(F32)
                                acc = acc + jnp.concatenate([po_v[g]] * (D // 128), axis=1) * w
                            beat(i + NA + NG)
                            return acc
                        acc = lax.fori_loop(0, NC1, loop_c, jnp.zeros((8, D), F32))
                        acc_v[...] += acc

                    if do_v and NC2:
                        with scope("idle"):
                            def loop_d(t, carry):
                                waitv(t + NA + NG + NC1)
                                beat(t + NA + NG + NC1)
                                return carry
                            lax.fori_loop(0, NC2, loop_d, 0)
                    return jnp.where(kslot == 2, 0, kslot + 1)

                kslot = lax.fori_loop(0, NH - 2, lambda h, ks: head(h, ks, True, True), jnp.int32(0))
                kslot = head(jnp.int32(NH - 2), kslot, False, True)
                cp_wg.start(priority=1)
                cp_wu.start(priority=1)
                for cp in cp_wd:
                    cp.start(priority=1)
                head(jnp.int32(NH - 1), kslot, False, False)

            pl.run_scoped(attn_scope, pltpu.SemaphoreType.DMA((3,)), pltpu.SemaphoreType.DMA((win,)))

            with scope("post"):
                attn = jnp.sum(acc_v[...], axis=0, keepdims=True)
                x1 = x_v[...].astype(F32) + mod_v[2] * attn
                h2 = (_ln(x1) * (1.0 + mod_v[4]) + mod_v[3]).astype(BF16)
            with scope("gate"):
                cp_wg.wait()
                g = jnp.dot(h2, wg_v[...], preferred_element_type=F32)
            with scope("up"):
                cp_wu.wait()
                u = jnp.dot(h2, wu_v[...], preferred_element_type=F32)
                act = (jax.nn.gelu(g, approximate=True) * u).astype(BF16)
            ffn = None
            for i in range(nwd - 1):
                with scope(f"down{i}"):
                    cp_wd[i].wait()
                    part = down_part(act, i)
                    ffn = part if ffn is None else ffn + part
            return x1, act, ffn

        x1, act, ffn = pl.run_scoped(ffn_scope, pltpu.SemaphoreType.DMA((nwd + 1,)))
        with scope("downlast"):
            wd_copy(nwd - 1, sem_last).wait()
            o_ref[...] = (x1 + mod_v[5] * (ffn + down_part(act, nwd - 1))).astype(o_ref.dtype)

    def fn(A_x, A_k_cache, A_v_cache, A_wq, A_wo, B_x, B_w_gate, B_w_up, B_w_down, c, w_mod):
        B, Sq, D = A_x.shape
        _, Hkv, SK, Dh = A_k_cache.shape
        assert B == 1 and Sq == 1 and Hkv == NH and Dh == DH
        W = min(4096, max(256, SK // 4))
        kt = jnp.swapaxes(A_k_cache, 2, 3).reshape(Hkv * NG, 8, SK)
        vt = jnp.swapaxes(A_v_cache, 2, 3).reshape(Hkv * NG, 8, SK)
        x2 = A_x.reshape(1, D)
        any_spec = pl.BlockSpec(memory_space=pl.ANY)
        out = pl.pallas_call(
            kernel,
            in_specs=[any_spec] * 10,
            out_specs=pl.BlockSpec(memory_space=pltpu.VMEM),
            out_shape=jax.ShapeDtypeStruct((1, D), A_x.dtype),
            scratch_shapes=[
                pltpu.VMEM((1, D), BF16), pltpu.VMEM((1, D), BF16),
                pltpu.VMEM(w_mod.shape, BF16), pltpu.VMEM(A_wq.shape, BF16), pltpu.VMEM((NH * NG, 8, D), BF16),
                pltpu.VMEM((3 * NG, 8, W + KPAD), BF16), pltpu.VMEM((2 * NG, 8, W), BF16),
                pltpu.VMEM(B_w_gate.shape, BF16), pltpu.VMEM(B_w_up.shape, BF16), pltpu.VMEM(B_w_down.shape, BF16),
                pltpu.VMEM((NH * Dh, 128), F32), pltpu.VMEM((8, W), F32),
                pltpu.VMEM((NG, 8, 128), F32),
                pltpu.VMEM((6, 1, D), F32), pltpu.VMEM((8, D), F32),
                pltpu.SemaphoreType.DMA,
            ],
            compiler_params=pltpu.CompilerParams(vmem_limit_bytes=100 * 1024 * 1024, disable_bounds_checks=nobc,
                                                 disable_semaphore_checks=nosc),
        )(x2, c, w_mod, A_wq, A_wo.reshape(NH * NG, 8, D), kt, vt, B_w_gate, B_w_up, B_w_down)
        return out.reshape(B, Sq, D)
    return fn


_impl = make()


@jax.jit
def pallas_adaLN_cond__sliding_block_cached__geglu_ffn__decode_kernel(
    A_x: jax.Array,
    A_k_cache: jax.Array,
    A_v_cache: jax.Array,
    A_wq: jax.Array,
    A_wo: jax.Array,
    B_x: jax.Array,
    B_w_gate: jax.Array,
    B_w_up: jax.Array,
    B_w_down: jax.Array,
    c: jax.Array,
    w_mod: jax.Array,
):
    return _impl(A_x, A_k_cache, A_v_cache, A_wq, A_wo, B_x, B_w_gate, B_w_up, B_w_down, c, w_mod)
```

```python
import functools

import jax
import jax.numpy as jnp
import numpy as np
from jax import lax
from jax.experimental import pallas as pl
from jax.experimental.pallas import tpu as pltpu

NH = 32
DH = 192
NG = DH // 8
WIN = 32
GP = 3
PC = 512
KPAD = 256
NW1 = 224
WD_CHUNKS = (512, 512, 256, 256)
BEATS_MOD, BEATS_Q, BEATS_T = 12, 20, 14
QBLK = 4

F32 = jnp.float32
BF16 = jnp.bfloat16
LOG2E = float(np.log2(np.e))


def _ln(x):
    m = jnp.mean(x, axis=-1, keepdims=True)
    d = x - m
    v = jnp.mean(d * d, axis=-1, keepdims=True)
    return d * lax.rsqrt(v + 1e-5)


def _tree_sum(xs):
    xs = list(xs)
    while len(xs) > 1:
        nxt = [xs[i] + xs[i + 1] for i in range(0, len(xs) - 1, 2)]
        if len(xs) % 2:
            nxt.append(xs[-1])
        xs = nxt
    return xs[0]


def _copy(src, dst, sem):
    return pltpu.make_async_copy(src, dst, sem)


def _kernel(x_hbm, c_hbm, wm_hbm, wq_hbm, wo_hbm, kt_hbm, vt_hbm, wg_hbm, wu_hbm, wd_hbm,
            o_ref,
            x_v, c_v, wm_v, wq_v, wo_v, k_v, v_v, wg_v, wu_v, wd_v,
            qb_v, s_v, po_v, mod_v, acc_v, sem_last):
    D = x_v.shape[1]
    SK = kt_hbm.shape[2]
    W = v_v.shape[2]
    RS = NG // GP
    P = RS * (W // PC)
    NT = W // 128
    RSH = int(np.log2(RS))
    JB = NT + 1
    JR = JB + NG
    JC = JR + 1
    NC = P - JC
    GC = NG // NC
    NR = D // 8
    nwd = len(WD_CHUNKS)
    offs = [int(o) for o in np.cumsum((0,) + WD_CHUNKS)]
    assert RS == 1 << RSH and P == 2 * WIN and NT == WIN and NC * GC == NG
    assert NR == P + WIN // 2 and WD_CHUNKS[0] == 16 * (P - NT) and offs[-1] == wd_v.shape[0]

    def kv_piece(src, dst, h, slot, j, sem):
        g = (j & (RS - 1)) * GP
        c = pl.multiple_of((j >> RSH) * PC, PC)
        return _copy(src.at[pl.ds(h * NG + g, GP), :, pl.ds(SK - W + c, PC)],
                     dst.at[pl.ds(slot * NG + g, GP), :, pl.ds(c, PC)], sem)

    def k_all(h, slot, sem):
        return _copy(kt_hbm.at[pl.ds(h * NG, NG), :, pl.ds(SK - W, W)],
                     k_v.at[pl.ds(slot * NG, NG), :, pl.ds(0, W)], sem)

    def row_piece(src, dst, i, rows, sem):
        r = pl.multiple_of(i * rows, rows)
        return _copy(src.at[pl.ds(r, rows)], dst.at[pl.ds(r, rows)], sem)

    def rows(src, dst, lo, n, sem):
        return _copy(src.at[pl.ds(lo, n)], dst.at[pl.ds(lo, n)], sem)

    def down_part(act, i):
        return jnp.dot(act[:, offs[i]:offs[i + 1]], wd_v[pl.ds(offs[i], WD_CHUNKS[i]), :],
                       preferred_element_type=F32)

    def ffn_scope(sem_f):
        def attn_scope(sem_k, sem_r):
            def ring(j):
                return sem_r.at[j & (WIN - 1)]

            def v_piece(h, slot, j):
                return kv_piece(vt_hbm, v_v, h, slot, j, ring(j))

            def k_piece(h, slot, j):
                return kv_piece(kt_hbm, k_v, h, slot, j, sem_k.at[slot])

            def prologue(sem_p):
                cp_c = _copy(c_hbm, c_v, sem_p.at[0])
                cp_x = _copy(x_hbm, x_v, sem_p.at[1])
                cp_c.start()
                cp_x.start()
                NQ = 6
                NWO = NH * NG // 2
                B1 = NR * NQ
                B2 = B1 + (NWO - NW1)
                B3 = B1 + NW1
                B4 = B3 + P
                assert B2 + 2 * P == B4 and B2 <= B3 and B1 % WIN == 0 and B3 % WIN == 0

                def w_piece(src, dst, b, sem):
                    g = lax.div(b, NQ)
                    pc = src.shape[1] // NQ
                    r = pl.multiple_of(g * 8, 8)
                    c = pl.multiple_of((b - g * NQ) * pc, 128)
                    return _copy(src.at[pl.ds(r, 8), pl.ds(c, pc)], dst.at[pl.ds(r, 8), pl.ds(c, pc)], sem)

                def p1_wq(b):
                    return w_piece(wq_hbm, wq_v, b, ring(b))

                def p1_wo(b):
                    return row_piece(wo_hbm, wo_v, b - B1, 2, ring(b))

                def p1_v0(b):
                    return v_piece(0, 0, b - B3)

                def p0_wm(b):
                    return w_piece(wm_hbm, wm_v, b, sem_p.at[2])

                def p0_wo(b):
                    return row_piece(wo_hbm, wo_v, b - B1 + NW1, 2, sem_p.at[3])

                def p0_k(b):
                    m = b - B2
                    hh = (m >= P).astype(jnp.int32)
                    return k_piece(hh, hh, m - hh * P)

                p1_tab = [(-WIN, None), (0, p1_wq), (B1, p1_wo), (B3, p1_v0)]
                p0_tab = [(0, p0_wm), (B1, p0_wo), (B2, p0_k)]
                cuts = sorted({0, WIN, B4} | {a + d for a, _ in p1_tab[1:] for d in (0, WIN)}
                              | {a for a, _ in p0_tab})

                def pick(tab, b):
                    return [f for a, f in tab if a <= b][-1]

                cur = [0]

                def beats(n):
                    lo, hi = cur[0], min(cur[0] + n, B4)
                    for a, e in zip(cuts[:-1], cuts[1:]):
                        s0, s1 = max(lo, a), min(hi, e)
                        if s1 <= s0:
                            continue

                        def body(b, carry, old=pick(p1_tab, a - WIN), p1=pick(p1_tab, a),
                                 p0=pick(p0_tab, a)):
                            if old is not None:
                                old(b - WIN).wait()
                            p1(b).start(priority=1)
                            p0(b).start(priority=0)
                            return carry
                        lax.fori_loop(s0, s1, body, 0)
                    cur[0] = hi

                beats(B1 + WIN)
                acc_v[...] = jnp.zeros(acc_v.shape, F32)

                cp_c.wait()
                cc = c_v[...].astype(F32)
                sc = (cc * jax.nn.sigmoid(cc)).astype(BF16)
                _copy(wm_hbm, wm_v, sem_p.at[2]).wait()
                for j in range(6):
                    md = jnp.dot(sc, wm_v[:, pl.ds(j * D, D)], preferred_element_type=F32)
                    mod_v[j] = md.astype(BF16).astype(F32)
                    beats(BEATS_MOD)
                cp_x.wait()
                h1 = (_ln(x_v[...].astype(F32)) * (1.0 + mod_v[1]) + mod_v[0]).astype(BF16)

                QB = NH * DH // QBLK
                scale = float(DH) ** -0.5 * LOG2E

                def q_mm(j):
                    q = jnp.dot(h1, wq_v[:, pl.ds(j * QB, QB)], preferred_element_type=F32)
                    return q.astype(BF16).astype(F32) * scale

                q = q_mm(0)
                beats(BEATS_T)
                for j in range(QBLK):
                    qn = q_mm(j + 1) if j + 1 < QBLK else None
                    for u in range(QB // 128):
                        row = q[:, u * 128:(u + 1) * 128]
                        qb_v[pl.ds(j * QB + u * 128, 128), :] = jnp.broadcast_to(row, (128, 128)).T
                    beats(BEATS_Q if j + 1 < QBLK else BEATS_T)
                    q = qn
                beats(B4)
                rows(wo_hbm, wo_v, 2 * NW1, NH * NG - 2 * NW1, sem_p.at[3]).wait()

            pl.run_scoped(prologue, pltpu.SemaphoreType.DMA((4,)))

            def head(h, kslot, p1, p0):
                vslot = h & 1

                def old(j0):
                    if j0 < WIN:
                        return lambda j: v_piece(h, vslot, j + WIN)
                    return lambda j: p1(j0 - WIN)(j - WIN)

                def wait(j0, j):
                    if j0 < WIN or p1 is not None:
                        old(j0)(j).wait()

                def start(j0, j):
                    if p1 is not None:
                        p1(j0)(j).start(priority=1)
                    if p0 is not None:
                        p0(j0)(j).start(priority=0)

                k_all(h, kslot, sem_k.at[kslot]).wait()

                qb = qb_v[pl.ds(pl.multiple_of(h * DH, 8), DH), :]
                qb = [qb[8 * g:8 * g + 8] for g in range(NG)]

                def loop_a(t, mx, j0):
                    wait(j0, t)
                    off = pl.multiple_of(t * 128, 128)
                    kt = k_v[pl.ds(kslot * NG, NG), :, pl.ds(off, 128)].astype(F32)
                    part = _tree_sum([kt[g] * qb[g] for g in range(NG)])
                    s = jnp.broadcast_to(jnp.sum(part, axis=0, keepdims=True), (8, 128))
                    s_v[:, pl.ds(off, 128)] = s
                    start(j0, t)
                    return jnp.maximum(mx, s)

                mx = jnp.full((8, 128), -jnp.inf, F32)
                for j0 in (0, WIN // 2):
                    mx = lax.fori_loop(j0, j0 + WIN // 2, functools.partial(loop_a, j0=j0), mx)
                m = jnp.max(mx, axis=1, keepdims=True)

                p = jnp.exp2(s_v[...] - m)
                wait(NT, jnp.int32(NT))
                start(NT, jnp.int32(NT))
                l = _tree_sum([p[:, t * 128:(t + 1) * 128] for t in range(NT)])
                inv_l = 1.0 / jnp.sum(l, axis=1, keepdims=True)

                def loop_b(g, carry):
                    wait(JB, g + JB)
                    prod = v_v[vslot * NG + g].astype(F32) * p
                    po_v[g] = _tree_sum([prod[:, t * 128:(t + 1) * 128] for t in range(NT)])
                    start(JB, g + JB)
                    return carry
                lax.fori_loop(0, NG, loop_b, 0)

                for g in range(NG):
                    o8 = jnp.sum(po_v[g], axis=1, keepdims=True) * inv_l
                    po_v[g] = jnp.broadcast_to(o8.astype(BF16).astype(F32), (8, 128))
                wait(JR, jnp.int32(JR))
                start(JR, jnp.int32(JR))

                def loop_c(i, acc):
                    wait(JC, i + JC)
                    for u in range(GC):
                        g = i * GC + u
                        w = wo_v[h * NG + g].astype(F32)
                        acc = acc + jnp.concatenate([po_v[g]] * (D // 128), axis=1) * w
                    start(JC, i + JC)
                    return acc
                acc_v[...] += lax.fori_loop(0, NC, loop_c, jnp.zeros((8, D), F32))
                return jnp.where(kslot == 2, 0, kslot + 1)

            def main_head(h, kslot):
                k_in = jnp.where(kslot == 0, 2, kslot - 1)
                v_in = 1 - (h & 1)
                return head(h, kslot,
                            lambda j0: (lambda j: v_piece(h + 1, v_in, j)),
                            lambda j0: (lambda j: k_piece(h + 2, k_in, j)))

            kslot = lax.fori_loop(0, NH - 2, main_head, jnp.int32(0))

            def wg_piece(off):
                return lambda j: row_piece(wg_hbm, wg_v, j + off, 8, sem_f.at[0])

            def wu_p0(off):
                return lambda j: row_piece(wu_hbm, wu_v, j + off, 8, sem_f.at[1])

            def wu_p1(j):
                return row_piece(wu_hbm, wu_v, j, 8, ring(j))

            def wd_p0(j):
                return row_piece(wd_hbm, wd_v, j - NT, 16, sem_f.at[2])

            def last_p0(j0):
                if j0 < WIN // 2:
                    return wg_piece(P)
                if j0 < WIN:
                    return wu_p0(P - WIN // 2)
                return wd_p0

            kslot = head(jnp.int32(NH - 2), kslot,
                         lambda j0: (lambda j: v_piece(NH - 1, 1, j)), lambda j0: wg_piece(0))
            head(jnp.int32(NH - 1), kslot, lambda j0: wu_p1, last_p0)
            cp_wd = [rows(wd_hbm, wd_v, offs[i], WD_CHUNKS[i],
                          sem_last if i == nwd - 1 else sem_f.at[2 + i]) for i in range(1, nwd)]
            for cp in cp_wd:
                cp.start(priority=1)

            attn = jnp.sum(acc_v[...], axis=0, keepdims=True)
            x1 = x_v[...].astype(F32) + mod_v[2] * attn
            h2 = (_ln(x1) * (1.0 + mod_v[4]) + mod_v[3]).astype(BF16)
            _copy(wg_hbm, wg_v, sem_f.at[0]).wait()
            g = jnp.dot(h2, wg_v[...], preferred_element_type=F32)

            def drain(j, carry):
                wu_p1(j).wait()
                return carry
            lax.fori_loop(P - WIN, P, drain, 0)
            rows(wu_hbm, wu_v, 8 * P, D - 8 * P, sem_f.at[1]).wait()
            return x1, h2, g

        x1, h2, g = pl.run_scoped(attn_scope, pltpu.SemaphoreType.DMA((3,)),
                                  pltpu.SemaphoreType.DMA((WIN,)))

        u = jnp.dot(h2, wu_v[...], preferred_element_type=F32)
        act = (jax.nn.gelu(g, approximate=True) * u).astype(BF16)
        ffn = None
        for i in range(nwd - 1):
            rows(wd_hbm, wd_v, offs[i], WD_CHUNKS[i], sem_f.at[2 + i]).wait()
            part = down_part(act, i)
            ffn = part if ffn is None else ffn + part
        return x1, act, ffn

    x1, act, ffn = pl.run_scoped(ffn_scope, pltpu.SemaphoreType.DMA((nwd + 1,)))
    rows(wd_hbm, wd_v, offs[-2], WD_CHUNKS[-1], sem_last).wait()
    o_ref[...] = (x1 + mod_v[5] * (ffn + down_part(act, nwd - 1))).astype(o_ref.dtype)


@jax.jit
def pallas_adaLN_cond__sliding_block_cached__geglu_ffn__decode_kernel(
    A_x: jax.Array,
    A_k_cache: jax.Array,
    A_v_cache: jax.Array,
    A_wq: jax.Array,
    A_wo: jax.Array,
    B_x: jax.Array,
    B_w_gate: jax.Array,
    B_w_up: jax.Array,
    B_w_down: jax.Array,
    c: jax.Array,
    w_mod: jax.Array,
):
    del B_x
    B, Sq, D = A_x.shape
    _, Hkv, SK, Dh = A_k_cache.shape
    assert (B, Sq, Hkv, Dh) == (1, 1, NH, DH), "decode kernel for a single query token"
    W = min(4096, max(256, SK // 4))
    kt = jnp.swapaxes(A_k_cache, 2, 3).reshape(NH * NG, 8, SK)
    vt = jnp.swapaxes(A_v_cache, 2, 3).reshape(NH * NG, 8, SK)
    wo = A_wo.reshape(NH * NG, 8, D)
    any_spec = pl.BlockSpec(memory_space=pl.ANY)
    out = pl.pallas_call(
        _kernel,
        in_specs=[any_spec] * 10,
        out_specs=pl.BlockSpec(memory_space=pltpu.VMEM),
        out_shape=jax.ShapeDtypeStruct((1, D), A_x.dtype),
        scratch_shapes=[
            pltpu.VMEM((1, D), BF16),
            pltpu.VMEM((1, D), BF16),
            pltpu.VMEM(w_mod.shape, BF16),
            pltpu.VMEM(A_wq.shape, BF16),
            pltpu.VMEM(wo.shape, BF16),
            pltpu.VMEM((3 * NG, 8, W + KPAD), BF16),
            pltpu.VMEM((2 * NG, 8, W), BF16),
            pltpu.VMEM(B_w_gate.shape, BF16),
            pltpu.VMEM(B_w_up.shape, BF16),
            pltpu.VMEM(B_w_down.shape, BF16),
            pltpu.VMEM((NH * DH, 128), F32),
            pltpu.VMEM((8, W), F32),
            pltpu.VMEM((NG, 8, 128), F32),
            pltpu.VMEM((6, 1, D), F32),
            pltpu.VMEM((8, D), F32),
            pltpu.SemaphoreType.DMA,
        ],
        compiler_params=pltpu.CompilerParams(
            vmem_limit_bytes=100 * 1024 * 1024,
            disable_bounds_checks=True,
        ),
    )(A_x.reshape(1, D), c, w_mod, A_wq, wo, kt, vt, B_w_gate, B_w_up, B_w_down)
    return out.reshape(B, Sq, D)
```

```python
import functools

import jax
import jax.numpy as jnp
import numpy as np
from jax import lax
from jax.experimental import pallas as pl
from jax.experimental.pallas import tpu as pltpu

NH = 32
DH = 192
NG = DH // 8
WIN = 32
GP = 3
PC = 512
KPAD = 256
NW1 = 144
WD_CHUNKS = (512, 512, 256, 256)
QBLK = 4
BEATS_0, BEATS_MOD, BEATS_Q, BEATS_T = 16, 8, 16, 10

F32 = jnp.float32
BF16 = jnp.bfloat16
LOG2E = float(np.log2(np.e))


def _ln(x):
    m = jnp.mean(x, axis=-1, keepdims=True)
    d = x - m
    v = jnp.mean(d * d, axis=-1, keepdims=True)
    return d * lax.rsqrt(v + 1e-5)


def _tree_sum(xs):
    xs = list(xs)
    while len(xs) > 1:
        nxt = [xs[i] + xs[i + 1] for i in range(0, len(xs) - 1, 2)]
        if len(xs) % 2:
            nxt.append(xs[-1])
        xs = nxt
    return xs[0]


def _copy(src, dst, sem):
    return pltpu.make_async_copy(src, dst, sem)


def _kernel(x_hbm, c_hbm, wm_hbm, wq_hbm, wo_hbm, kt_hbm, vt_hbm, wg_hbm, wu_hbm, wd_hbm,
            o_ref,
            x_v, c_v, wm_v, wq_v, wo_v, k_v, v_v, wg_v, wu_v, wd_v,
            qb_v, s_v, po_v, mod_v, acc_v, sem_last):
    D = x_v.shape[1]
    SK = kt_hbm.shape[2]
    W = v_v.shape[2]
    RS = NG // GP
    P = RS * (W // PC)
    NT = W // 128
    RSH = int(np.log2(RS))
    JB = NT + 1
    JR = JB + NG
    JC = JR + 1
    NC = P - JC
    GC = NG // NC
    NR = D // 8
    nwd = len(WD_CHUNKS)
    offs = [int(o) for o in np.cumsum((0,) + WD_CHUNKS)]
    assert RS == 1 << RSH and P == 2 * WIN and NT == WIN and NC * GC == NG
    assert NR == P + WIN // 2 and WD_CHUNKS[0] == 16 * (P - NT) and offs[-1] == wd_v.shape[0]

    def kv_piece(src, dst, h, slot, j, sem):
        g = (j & (RS - 1)) * GP
        c = pl.multiple_of((j >> RSH) * PC, PC)
        return _copy(src.at[pl.ds(h * NG + g, GP), :, pl.ds(SK - W + c, PC)],
                     dst.at[pl.ds(slot * NG + g, GP), :, pl.ds(c, PC)], sem)

    def k_all(h, slot, sem):
        return _copy(kt_hbm.at[pl.ds(h * NG, NG), :, pl.ds(SK - W, W)],
                     k_v.at[pl.ds(slot * NG, NG), :, pl.ds(0, W)], sem)

    def row_piece(src, dst, i, rows, sem):
        r = pl.multiple_of(i * rows, rows)
        return _copy(src.at[pl.ds(r, rows)], dst.at[pl.ds(r, rows)], sem)

    def rows(src, dst, lo, n, sem):
        return _copy(src.at[pl.ds(lo, n)], dst.at[pl.ds(lo, n)], sem)

    def down_part(act, i):
        return jnp.dot(act[:, offs[i]:offs[i + 1]], wd_v[pl.ds(offs[i], WD_CHUNKS[i]), :],
                       preferred_element_type=F32)

    def ffn_scope(sem_f):
        def attn_scope(sem_k, sem_r):
            def ring(j):
                return sem_r.at[j & (WIN - 1)]

            def v_piece(h, slot, j):
                return kv_piece(vt_hbm, v_v, h, slot, j, ring(j))

            def k_piece(h, slot, j):
                return kv_piece(kt_hbm, k_v, h, slot, j, sem_k.at[slot])

            def prologue(sem_p):
                cp_c = _copy(c_hbm, c_v, sem_p.at[0])
                cp_x = _copy(x_hbm, x_v, sem_p.at[1])
                cp_c.start()
                cp_x.start()
                NB = 8
                NQ, NM = 4, 2
                PQ, PM = NR * NQ, NR * NM
                NWO = NH * NG // 2
                NW0 = NWO - NW1
                B1 = PQ
                B3 = B1 + NW1
                B4 = B3 + P
                C1 = PM
                C2 = C1 + NW0
                assert C2 + 2 * P == B4 and NW1 % NB == 0 and NW0 % NB == 0 and C1 + WIN <= B1
                OFF = (-B3) % WIN

                def w_piece(src, dst, b, ncol, sem):
                    i = b >> 3
                    sh = int(np.log2(ncol))
                    assert ncol == 1 << sh
                    pc = src.shape[1] // ncol
                    r = pl.multiple_of(((b & (NB - 1)) * (NR // NB) + (i >> sh)) * 8, 8)
                    c = pl.multiple_of((i & (ncol - 1)) * pc, 128)
                    return _copy(src.at[pl.ds(r, 8), pl.ds(c, pc)], dst.at[pl.ds(r, 8), pl.ds(c, pc)], sem)

                def wo_piece(i, base, n, sem):
                    return row_piece(wo_hbm, wo_v, base + (i & (NB - 1)) * (n // NB) + (i >> 3), 2, sem)

                def p1_wq(b):
                    return w_piece(wq_hbm, wq_v, b, NQ, ring(b + OFF))

                def p1_wo(b):
                    return wo_piece(b - B1, 0, NW1, ring(b + OFF))

                def p1_v0(b):
                    return v_piece(0, 0, b - B3)

                def p0_wm(b):
                    return w_piece(wm_hbm, wm_v, b, NM, sem_p.at[2])

                def p0_wo(b):
                    return wo_piece(b - C1, NW1, NW0, sem_p.at[3])

                def p0_k(b):
                    m = b - C2
                    hh = (m >= P).astype(jnp.int32)
                    return k_piece(hh, hh, m - hh * P)

                p1_tab = [(-WIN, None), (0, p1_wq), (B1, p1_wo), (B3, p1_v0)]
                p0_tab = [(0, p0_wm), (C1, p0_wo), (C2, p0_k)]
                cuts = sorted({0, WIN, B4} | {a + d for a, _ in p1_tab[1:] for d in (0, WIN)}
                              | {a for a, _ in p0_tab})

                def pick(tab, b):
                    return [f for a, f in tab if a <= b][-1]

                cur = [0]

                def beats(n):
                    lo, hi = cur[0], min(cur[0] + n, B4)
                    for a, e in zip(cuts[:-1], cuts[1:]):
                        s0, s1 = max(lo, a), min(hi, e)
                        if s1 <= s0:
                            continue

                        def body(b, carry, old=pick(p1_tab, a - WIN), p1=pick(p1_tab, a),
                                 p0=pick(p0_tab, a)):
                            if old is not None:
                                old(b - WIN).wait()
                            p1(b).start(priority=1)
                            p0(b).start(priority=0)
                            return carry
                        lax.fori_loop(s0, s1, body, 0)
                    cur[0] = hi

                beats(C1 + BEATS_0)
                acc_v[...] = jnp.zeros(acc_v.shape, F32)

                cp_c.wait()
                cc = c_v[...].astype(F32)
                sc = (cc * jax.nn.sigmoid(cc)).astype(BF16)
                _copy(wm_hbm, wm_v, sem_p.at[2]).wait()
                for j in range(6):
                    md = jnp.dot(sc, wm_v[:, pl.ds(j * D, D)], preferred_element_type=F32)
                    mod_v[j] = md.astype(BF16).astype(F32)
                    beats(BEATS_MOD)
                cp_x.wait()
                h1 = (_ln(x_v[...].astype(F32)) * (1.0 + mod_v[1]) + mod_v[0]).astype(BF16)
                beats(B1 + WIN - cur[0])

                QB = NH * DH // QBLK
                scale = float(DH) ** -0.5 * LOG2E

                def q_mm(j):
                    q = jnp.dot(h1, wq_v[:, pl.ds(j * QB, QB)], preferred_element_type=F32)
                    return q.astype(BF16).astype(F32) * scale

                q = q_mm(0)
                beats(BEATS_T)
                for j in range(QBLK):
                    qn = q_mm(j + 1) if j + 1 < QBLK else None
                    for u in range(QB // 128):
                        row = q[:, u * 128:(u + 1) * 128]
                        qb_v[pl.ds(j * QB + u * 128, 128), :] = jnp.broadcast_to(row, (128, 128)).T
                    beats(BEATS_Q if j + 1 < QBLK else BEATS_T)
                    q = qn
                beats(B4)
                rows(wo_hbm, wo_v, 2 * NW1, 2 * NW0, sem_p.at[3]).wait()

            pl.run_scoped(prologue, pltpu.SemaphoreType.DMA((4,)))

            def head(h, kslot, p1, p0):
                vslot = h & 1

                def old(j0):
                    if j0 < WIN:
                        return lambda j: v_piece(h, vslot, j + WIN)
                    return lambda j: p1(j0 - WIN)(j - WIN)

                def wait(j0, j):
                    if j0 < WIN or p1 is not None:
                        old(j0)(j).wait()

                def start(j0, j):
                    if p1 is not None:
                        p1(j0)(j).start(priority=1)
                    if p0 is not None:
                        p0(j0)(j).start(priority=0)

                k_all(h, kslot, sem_k.at[kslot]).wait()

                qb = qb_v[pl.ds(pl.multiple_of(h * DH, 8), DH), :]
                qb = [qb[8 * g:8 * g + 8] for g in range(NG)]

                def loop_a(t, mx, j0):
                    wait(j0, t)
                    off = pl.multiple_of(t * 128, 128)
                    kt = k_v[pl.ds(kslot * NG, NG), :, pl.ds(off, 128)].astype(F32)
                    part = _tree_sum([kt[g] * qb[g] for g in range(NG)])
                    s = jnp.broadcast_to(jnp.sum(part, axis=0, keepdims=True), (8, 128))
                    s_v[:, pl.ds(off, 128)] = s
                    start(j0, t)
                    return jnp.maximum(mx, s)

                mx = jnp.full((8, 128), -jnp.inf, F32)
                for j0 in (0, WIN // 2):
                    mx = lax.fori_loop(j0, j0 + WIN // 2, functools.partial(loop_a, j0=j0), mx)
                m = jnp.max(mx, axis=1, keepdims=True)

                p = jnp.exp2(s_v[...] - m)
                wait(NT, jnp.int32(NT))
                start(NT, jnp.int32(NT))
                l = _tree_sum([p[:, t * 128:(t + 1) * 128] for t in range(NT)])
                inv_l = 1.0 / jnp.sum(l, axis=1, keepdims=True)

                def loop_b(g, carry):
                    wait(JB, g + JB)
                    prod = v_v[vslot * NG + g].astype(F32) * p
                    po_v[g] = _tree_sum([prod[:, t * 128:(t + 1) * 128] for t in range(NT)])
                    start(JB, g + JB)
                    return carry
                lax.fori_loop(0, NG, loop_b, 0)

                for g in range(NG):
                    o8 = jnp.sum(po_v[g], axis=1, keepdims=True) * inv_l
                    po_v[g] = jnp.broadcast_to(o8.astype(BF16).astype(F32), (8, 128))
                wait(JR, jnp.int32(JR))
                start(JR, jnp.int32(JR))

                def loop_c(i, acc):
                    wait(JC, i + JC)
                    for u in range(GC):
                        g = i * GC + u
                        w = wo_v[h * NG + g].astype(F32)
                        acc = acc + jnp.concatenate([po_v[g]] * (D // 128), axis=1) * w
                    start(JC, i + JC)
                    return acc
                acc_v[...] += lax.fori_loop(0, NC, loop_c, jnp.zeros((8, D), F32))
                return jnp.where(kslot == 2, 0, kslot + 1)

            def main_head(h, kslot):
                k_in = jnp.where(kslot == 0, 2, kslot - 1)
                v_in = 1 - (h & 1)
                return head(h, kslot,
                            lambda j0: (lambda j: v_piece(h + 1, v_in, j)),
                            lambda j0: (lambda j: k_piece(h + 2, k_in, j)))

            kslot = lax.fori_loop(0, NH - 2, main_head, jnp.int32(0))

            class _Either:
                def __init__(self, j, i, sem_g, sem_u):
                    self.j, self.i, self.sems = j, i, (sem_g, sem_u)

                def start(self, priority):
                    pl.when((self.j & 1) == 0)(
                        lambda: row_piece(wg_hbm, wg_v, self.i, 8, self.sems[0]).start(priority=priority))
                    pl.when((self.j & 1) == 1)(
                        lambda: row_piece(wu_hbm, wu_v, self.i, 8, self.sems[1]).start(priority=priority))

                def wait(self):
                    pl.when((self.j & 1) == 0)(lambda: row_piece(wg_hbm, wg_v, self.i, 8, self.sems[0]).wait())
                    pl.when((self.j & 1) == 1)(lambda: row_piece(wu_hbm, wu_v, self.i, 8, self.sems[1]).wait())

            def gu_p0(base):
                return lambda j: _Either(j, base + (j >> 1), sem_f.at[0], sem_f.at[1])

            def gu_p1(j):
                return _Either(j, P // 2 + (j >> 1), ring(j), ring(j))

            def wd_p0(j):
                return row_piece(wd_hbm, wd_v, j - NT, 16, sem_f.at[2])

            kslot = head(jnp.int32(NH - 2), kslot,
                         lambda j0: (lambda j: v_piece(NH - 1, 1, j)), lambda j0: gu_p0(0))
            head(jnp.int32(NH - 1), kslot, lambda j0: gu_p1, lambda j0: gu_p0(P) if j0 < WIN else wd_p0)
            cp_wd = [rows(wd_hbm, wd_v, offs[i], WD_CHUNKS[i],
                          sem_last if i == nwd - 1 else sem_f.at[2 + i]) for i in range(1, nwd)]
            for cp in cp_wd:
                cp.start(priority=1)

            attn = jnp.sum(acc_v[...], axis=0, keepdims=True)
            x1 = x_v[...].astype(F32) + mod_v[2] * attn
            h2 = (_ln(x1) * (1.0 + mod_v[4]) + mod_v[3]).astype(BF16)
            def drain(lo, hi):
                def body(j, carry):
                    gu_p1(j).wait()
                    return carry
                lax.fori_loop(lo, hi, body, 0)
            for src, dst, sem in ((wg_hbm, wg_v, sem_f.at[0]), (wu_hbm, wu_v, sem_f.at[1])):
                rows(src, dst, 0, 4 * P, sem).wait()
                rows(src, dst, 8 * P, D - 8 * P, sem).wait()
            drain(P - WIN, P)
            g = jnp.dot(h2, wg_v[...], preferred_element_type=F32)
            return x1, h2, g

        x1, h2, g = pl.run_scoped(attn_scope, pltpu.SemaphoreType.DMA((3,)),
                                  pltpu.SemaphoreType.DMA((WIN,)))

        u = jnp.dot(h2, wu_v[...], preferred_element_type=F32)
        act = (jax.nn.gelu(g, approximate=True) * u).astype(BF16)
        ffn = None
        for i in range(nwd - 1):
            rows(wd_hbm, wd_v, offs[i], WD_CHUNKS[i], sem_f.at[2 + i]).wait()
            part = down_part(act, i)
            ffn = part if ffn is None else ffn + part
        return x1, act, ffn

    x1, act, ffn = pl.run_scoped(ffn_scope, pltpu.SemaphoreType.DMA((nwd + 1,)))
    rows(wd_hbm, wd_v, offs[-2], WD_CHUNKS[-1], sem_last).wait()
    o_ref[...] = (x1 + mod_v[5] * (ffn + down_part(act, nwd - 1))).astype(o_ref.dtype)


@jax.jit
def pallas_adaLN_cond__sliding_block_cached__geglu_ffn__decode_kernel(
    A_x: jax.Array,
    A_k_cache: jax.Array,
    A_v_cache: jax.Array,
    A_wq: jax.Array,
    A_wo: jax.Array,
    B_x: jax.Array,
    B_w_gate: jax.Array,
    B_w_up: jax.Array,
    B_w_down: jax.Array,
    c: jax.Array,
    w_mod: jax.Array,
):
    del B_x
    B, Sq, D = A_x.shape
    _, Hkv, SK, Dh = A_k_cache.shape
    assert (B, Sq, Hkv, Dh) == (1, 1, NH, DH), "decode kernel for a single query token"
    W = min(4096, max(256, SK // 4))
    kt = jnp.swapaxes(A_k_cache, 2, 3).reshape(NH * NG, 8, SK)
    vt = jnp.swapaxes(A_v_cache, 2, 3).reshape(NH * NG, 8, SK)
    wo = A_wo.reshape(NH * NG, 8, D)
    any_spec = pl.BlockSpec(memory_space=pl.ANY)
    out = pl.pallas_call(
        _kernel,
        in_specs=[any_spec] * 10,
        out_specs=pl.BlockSpec(memory_space=pltpu.VMEM),
        out_shape=jax.ShapeDtypeStruct((1, D), A_x.dtype),
        scratch_shapes=[
            pltpu.VMEM((1, D), BF16),
            pltpu.VMEM((1, D), BF16),
            pltpu.VMEM(w_mod.shape, BF16),
            pltpu.VMEM(A_wq.shape, BF16),
            pltpu.VMEM(wo.shape, BF16),
            pltpu.VMEM((3 * NG, 8, W + KPAD), BF16),
            pltpu.VMEM((2 * NG, 8, W), BF16),
            pltpu.VMEM(B_w_gate.shape, BF16),
            pltpu.VMEM(B_w_up.shape, BF16),
            pltpu.VMEM(B_w_down.shape, BF16),
            pltpu.VMEM((NH * DH, 128), F32),
            pltpu.VMEM((8, W), F32),
            pltpu.VMEM((NG, 8, 128), F32),
            pltpu.VMEM((6, 1, D), F32),
            pltpu.VMEM((8, D), F32),
            pltpu.SemaphoreType.DMA,
        ],
        compiler_params=pltpu.CompilerParams(
            vmem_limit_bytes=100 * 1024 * 1024,
            disable_bounds_checks=True,
        ),
    )(A_x.reshape(1, D), c, w_mod, A_wq, wo, kt, vt, B_w_gate, B_w_up, B_w_down)
    return out.reshape(B, Sq, D)
```

```python
import functools

import jax
import jax.numpy as jnp
import numpy as np
from jax import lax
from jax.experimental import pallas as pl
from jax.experimental.pallas import tpu as pltpu

NH = 32
DH = 192
NG = DH // 8
WIN = 32
GP = 3
PC = 512
KPAD = 256
NW1 = 144
WD_CHUNKS = (512, 512, 256, 256)
QBLK = 4
BEATS_0, BEATS_MOD, BEATS_Q, BEATS_T = 16, 8, 16, 10

F32 = jnp.float32
BF16 = jnp.bfloat16
LOG2E = float(np.log2(np.e))


def _ln(x):
    m = jnp.mean(x, axis=-1, keepdims=True)
    d = x - m
    v = jnp.mean(d * d, axis=-1, keepdims=True)
    return d * lax.rsqrt(v + 1e-5)


def _tree_sum(xs):
    xs = list(xs)
    while len(xs) > 1:
        nxt = [xs[i] + xs[i + 1] for i in range(0, len(xs) - 1, 2)]
        if len(xs) % 2:
            nxt.append(xs[-1])
        xs = nxt
    return xs[0]


def _copy(src, dst, sem):
    return pltpu.make_async_copy(src, dst, sem)


def _kernel(x_hbm, c_hbm, wm_hbm, wq_hbm, wo_hbm, kt_hbm, vt_hbm, wg_hbm, wu_hbm, wd_hbm,
            o_ref,
            x_v, c_v, wm_v, wq_v, wo_v, k_v, v_v, wg_v, wu_v, wd_v,
            qb_v, s_v, po_v, mod_v, acc_v, sem_last):
    D = x_v.shape[1]
    SK = kt_hbm.shape[2]
    W = v_v.shape[2]
    RS = NG // GP
    P = RS * (W // PC)
    NT = W // 128
    RSH = int(np.log2(RS))
    JB = NT + 1
    JR = JB + NG
    JC = JR + 1
    NC = P - JC
    GC = NG // NC
    NR = D // 8
    nwd = len(WD_CHUNKS)
    offs = [int(o) for o in np.cumsum((0,) + WD_CHUNKS)]
    assert RS == 1 << RSH and P == 2 * WIN and NT == WIN and NC * GC == NG
    assert NR == P + WIN // 2 and WD_CHUNKS[0] == 16 * (P - NT) and offs[-1] == wd_v.shape[0]

    def kv_piece(src, dst, h, slot, j, sem):
        g = (j & (RS - 1)) * GP
        c = pl.multiple_of((j >> RSH) * PC, PC)
        return _copy(src.at[pl.ds(h * NG + g, GP), :, pl.ds(SK - W + c, PC)],
                     dst.at[pl.ds(slot * NG + g, GP), :, pl.ds(c, PC)], sem)

    def k_all(h, slot, sem):
        return _copy(kt_hbm.at[pl.ds(h * NG, NG), :, pl.ds(SK - W, W)],
                     k_v.at[pl.ds(slot * NG, NG), :, pl.ds(0, W)], sem)

    def row_piece(src, dst, i, rows, sem):
        r = pl.multiple_of(i * rows, rows)
        return _copy(src.at[pl.ds(r, rows)], dst.at[pl.ds(r, rows)], sem)

    def rows(src, dst, lo, n, sem):
        return _copy(src.at[pl.ds(lo, n)], dst.at[pl.ds(lo, n)], sem)

    def down_part(act, i):
        return jnp.dot(act[:, offs[i]:offs[i + 1]], wd_v[pl.ds(offs[i], WD_CHUNKS[i]), :],
                       preferred_element_type=F32)

    def ffn_scope(sem_f):
        def attn_scope(sem_k, sem_r):
            def ring(j):
                return sem_r.at[j & (WIN - 1)]

            def v_piece(h, slot, j):
                return kv_piece(vt_hbm, v_v, h, slot, j, ring(j))

            def k_piece(h, slot, j):
                return kv_piece(kt_hbm, k_v, h, slot, j, sem_k.at[slot])

            def prologue(sem_p):
                cp_c = _copy(c_hbm, c_v, sem_p.at[0])
                cp_x = _copy(x_hbm, x_v, sem_p.at[1])
                cp_c.start()
                cp_x.start()
                NB = 8
                NQ, NM = 4, 2
                PQ, PM = NR * NQ, NR * NM
                NWO = NH * NG // 2
                NW0 = NWO - NW1
                B1 = PQ
                B3 = B1 + NW1
                B4 = B3 + P
                C1 = PM
                C2 = C1 + NW0
                assert C2 + 2 * P == B4 and NW1 % NB == 0 and NW0 % NB == 0 and C1 + WIN <= B1
                OFF = (-B3) % WIN

                def w_piece(src, dst, b, ncol, sem):
                    i = b >> 3
                    sh = int(np.log2(ncol))
                    assert ncol == 1 << sh
                    pc = src.shape[1] // ncol
                    r = pl.multiple_of(((b & (NB - 1)) * (NR // NB) + (i >> sh)) * 8, 8)
                    c = pl.multiple_of((i & (ncol - 1)) * pc, 128)
                    return _copy(src.at[pl.ds(r, 8), pl.ds(c, pc)], dst.at[pl.ds(r, 8), pl.ds(c, pc)], sem)

                def wo_piece(i, base, n, sem):
                    return row_piece(wo_hbm, wo_v, base + (i & (NB - 1)) * (n // NB) + (i >> 3), 2, sem)

                def p1_wq(b):
                    return w_piece(wq_hbm, wq_v, b, NQ, ring(b + OFF))

                def p1_wo(b):
                    return wo_piece(b - B1, 0, NW1, ring(b + OFF))

                def p1_v0(b):
                    return v_piece(0, 0, b - B3)

                def p0_wm(b):
                    return w_piece(wm_hbm, wm_v, b, NM, sem_p.at[2])

                def p0_wo(b):
                    return wo_piece(b - C1, NW1, NW0, sem_p.at[3])

                def p0_k(b):
                    m = b - C2
                    hh = (m >= P).astype(jnp.int32)
                    return k_piece(hh, hh, m - hh * P)

                p1_tab = [(-WIN, None), (0, p1_wq), (B1, p1_wo), (B3, p1_v0)]
                p0_tab = [(0, p0_wm), (C1, p0_wo), (C2, p0_k)]
                cuts = sorted({0, WIN, B4} | {a + d for a, _ in p1_tab[1:] for d in (0, WIN)}
                              | {a for a, _ in p0_tab})

                def pick(tab, b):
                    return [f for a, f in tab if a <= b][-1]

                cur = [0]

                def beats(n):
                    lo, hi = cur[0], min(cur[0] + n, B4)
                    for a, e in zip(cuts[:-1], cuts[1:]):
                        s0, s1 = max(lo, a), min(hi, e)
                        if s1 <= s0:
                            continue

                        def body(b, carry, old=pick(p1_tab, a - WIN), p1=pick(p1_tab, a),
                                 p0=pick(p0_tab, a)):
                            if old is not None:
                                old(b - WIN).wait()
                            p1(b).start(priority=1)
                            p0(b).start(priority=0)
                            return carry
                        lax.fori_loop(s0, s1, body, 0)
                    cur[0] = hi

                beats(C1 + BEATS_0)
                acc_v[...] = jnp.zeros(acc_v.shape, F32)

                cp_c.wait()
                cc = c_v[...].astype(F32)
                sc = (cc * jax.nn.sigmoid(cc)).astype(BF16)
                _copy(wm_hbm, wm_v, sem_p.at[2]).wait()
                for j in range(6):
                    md = jnp.dot(sc, wm_v[:, pl.ds(j * D, D)], preferred_element_type=F32)
                    mod_v[j] = md.astype(BF16).astype(F32)
                    beats(BEATS_MOD)
                cp_x.wait()
                h1 = (_ln(x_v[...].astype(F32)) * (1.0 + mod_v[1]) + mod_v[0]).astype(BF16)
                beats(B1 + WIN - cur[0])

                QB = NH * DH // QBLK
                scale = float(DH) ** -0.5 * LOG2E

                def q_mm(j):
                    q = jnp.dot(h1, wq_v[:, pl.ds(j * QB, QB)], preferred_element_type=F32)
                    return q.astype(BF16).astype(F32) * scale

                q = q_mm(0)
                beats(BEATS_T)
                for j in range(QBLK):
                    qn = q_mm(j + 1) if j + 1 < QBLK else None
                    for u in range(QB // 128):
                        row = q[:, u * 128:(u + 1) * 128]
                        qb_v[pl.ds(j * QB + u * 128, 128), :] = jnp.broadcast_to(row, (128, 128)).T
                    beats(BEATS_Q if j + 1 < QBLK else BEATS_T)
                    q = qn
                beats(B4)
                rows(wo_hbm, wo_v, 2 * NW1, 2 * NW0, sem_p.at[3]).wait()

            pl.run_scoped(prologue, pltpu.SemaphoreType.DMA((4,)))

            def head(h, kslot, p1, p0):
                vslot = h & 1

                def old(j0):
                    if j0 < WIN:
                        return lambda j: v_piece(h, vslot, j + WIN)
                    return lambda j: p1(j0 - WIN)(j - WIN)

                def wait(j0, j):
                    if j0 < WIN or p1 is not None:
                        old(j0)(j).wait()

                def start(j0, j):
                    if p1 is not None:
                        p1(j0)(j).start(priority=1)
                    if p0 is not None:
                        p0(j0)(j).start(priority=0)

                k_all(h, kslot, sem_k.at[kslot]).wait()

                qb = qb_v[pl.ds(pl.multiple_of(h * DH, 8), DH), :]
                qb = [qb[8 * g:8 * g + 8] for g in range(NG)]

                def loop_a(t, mx, j0):
                    wait(j0, t)
                    off = pl.multiple_of(t * 128, 128)
                    kt = k_v[pl.ds(kslot * NG, NG), :, pl.ds(off, 128)].astype(F32)
                    part = _tree_sum([kt[g] * qb[g] for g in range(NG)])
                    s = jnp.broadcast_to(jnp.sum(part, axis=0, keepdims=True), (8, 128))
                    s_v[:, pl.ds(off, 128)] = s
                    start(j0, t)
                    return jnp.maximum(mx, s)

                mx = jnp.full((8, 128), -jnp.inf, F32)
                for j0 in (0, WIN // 2):
                    mx = lax.fori_loop(j0, j0 + WIN // 2, functools.partial(loop_a, j0=j0), mx)
                m = jnp.max(mx, axis=1, keepdims=True)

                p = jnp.exp2(s_v[...] - m)
                wait(NT, jnp.int32(NT))
                start(NT, jnp.int32(NT))
                l = _tree_sum([p[:, t * 128:(t + 1) * 128] for t in range(NT)])
                inv_l = 1.0 / jnp.sum(l, axis=1, keepdims=True)

                def loop_b(g, carry):
                    wait(JB, g + JB)
                    prod = v_v[vslot * NG + g].astype(F32) * p
                    po_v[g] = _tree_sum([prod[:, t * 128:(t + 1) * 128] for t in range(NT)])
                    start(JB, g + JB)
                    return carry
                lax.fori_loop(0, NG, loop_b, 0)

                for g in range(NG):
                    o8 = jnp.sum(po_v[g], axis=1, keepdims=True) * inv_l
                    po_v[g] = jnp.broadcast_to(o8.astype(BF16).astype(F32), (8, 128))
                wait(JR, jnp.int32(JR))
                start(JR, jnp.int32(JR))

                def loop_c(i, acc):
                    wait(JC, i + JC)
                    for u in range(GC):
                        g = i * GC + u
                        w = wo_v[h * NG + g].astype(F32)
                        acc = acc + jnp.concatenate([po_v[g]] * (D // 128), axis=1) * w
                    start(JC, i + JC)
                    return acc
                acc_v[...] += lax.fori_loop(0, NC, loop_c, jnp.zeros((8, D), F32))
                return jnp.where(kslot == 2, 0, kslot + 1)

            def main_head(h, kslot):
                k_in = jnp.where(kslot == 0, 2, kslot - 1)
                v_in = 1 - (h & 1)
                return head(h, kslot,
                            lambda j0: (lambda j: v_piece(h + 1, v_in, j)),
                            lambda j0: (lambda j: k_piece(h + 2, k_in, j)))

            kslot = lax.fori_loop(0, NH - 2, main_head, jnp.int32(0))

            class _Either:
                def __init__(self, j, i, sem_g, sem_u):
                    self.j, self.i, self.sems = j, i, (sem_g, sem_u)

                def start(self, priority):
                    pl.when((self.j & 1) == 0)(
                        lambda: row_piece(wg_hbm, wg_v, self.i, 8, self.sems[0]).start(priority=priority))
                    pl.when((self.j & 1) == 1)(
                        lambda: row_piece(wu_hbm, wu_v, self.i, 8, self.sems[1]).start(priority=priority))

                def wait(self):
                    pl.when((self.j & 1) == 0)(lambda: row_piece(wg_hbm, wg_v, self.i, 8, self.sems[0]).wait())
                    pl.when((self.j & 1) == 1)(lambda: row_piece(wu_hbm, wu_v, self.i, 8, self.sems[1]).wait())

            def gu_p0(base):
                return lambda j: _Either(j, base + (j >> 1), sem_f.at[0], sem_f.at[1])

            def gu_p1(j):
                return _Either(j, P // 2 + (j >> 1), ring(j), ring(j))

            def wd_p0(j):
                return row_piece(wd_hbm, wd_v, j - NT, 16, sem_f.at[2])

            kslot = head(jnp.int32(NH - 2), kslot,
                         lambda j0: (lambda j: v_piece(NH - 1, 1, j)), lambda j0: gu_p0(0))
            head(jnp.int32(NH - 1), kslot, lambda j0: gu_p1, lambda j0: gu_p0(P) if j0 < WIN else wd_p0)
            cp_wd = [rows(wd_hbm, wd_v, offs[i], WD_CHUNKS[i],
                          sem_last if i == nwd - 1 else sem_f.at[2 + i]) for i in range(1, nwd)]
            for cp in cp_wd:
                cp.start(priority=1)

            attn = jnp.sum(acc_v[...], axis=0, keepdims=True)
            x1 = x_v[...].astype(F32) + mod_v[2] * attn
            h2 = (_ln(x1) * (1.0 + mod_v[4]) + mod_v[3]).astype(BF16)
            def drain(lo, hi):
                def body(j, carry):
                    gu_p1(j).wait()
                    return carry
                lax.fori_loop(lo, hi, body, 0)
            for src, dst, sem in ((wg_hbm, wg_v, sem_f.at[0]), (wu_hbm, wu_v, sem_f.at[1])):
                rows(src, dst, 0, 4 * P, sem).wait()
                rows(src, dst, 8 * P, D - 8 * P, sem).wait()
            drain(P - WIN, P)
            g = jnp.dot(h2, wg_v[...], preferred_element_type=F32)
            return x1, h2, g

        x1, h2, g = pl.run_scoped(attn_scope, pltpu.SemaphoreType.DMA((3,)),
                                  pltpu.SemaphoreType.DMA((WIN,)))

        u = jnp.dot(h2, wu_v[...], preferred_element_type=F32)
        act = (jax.nn.gelu(g, approximate=True) * u).astype(BF16)
        ffn = None
        for i in range(nwd - 1):
            rows(wd_hbm, wd_v, offs[i], WD_CHUNKS[i], sem_f.at[2 + i]).wait()
            part = down_part(act, i)
            ffn = part if ffn is None else ffn + part
        return x1, act, ffn

    x1, act, ffn = pl.run_scoped(ffn_scope, pltpu.SemaphoreType.DMA((nwd + 1,)))
    rows(wd_hbm, wd_v, offs[-2], WD_CHUNKS[-1], sem_last).wait()
    o_ref[...] = (x1 + mod_v[5] * (ffn + down_part(act, nwd - 1))).astype(o_ref.dtype)


@jax.jit
def pallas_adaLN_cond__sliding_block_cached__geglu_ffn__decode_kernel(
    A_x: jax.Array,
    A_k_cache: jax.Array,
    A_v_cache: jax.Array,
    A_wq: jax.Array,
    A_wo: jax.Array,
    B_x: jax.Array,
    B_w_gate: jax.Array,
    B_w_up: jax.Array,
    B_w_down: jax.Array,
    c: jax.Array,
    w_mod: jax.Array,
):
    del B_x
    B, Sq, D = A_x.shape
    _, Hkv, SK, Dh = A_k_cache.shape
    assert (B, Sq, Hkv, Dh) == (1, 1, NH, DH), "decode kernel for a single query token"
    W = min(4096, max(256, SK // 4))
    kt = jnp.swapaxes(A_k_cache, 2, 3).reshape(NH * NG, 8, SK)
    vt = jnp.swapaxes(A_v_cache, 2, 3).reshape(NH * NG, 8, SK)
    wo = A_wo.reshape(NH * NG, 8, D)
    any_spec = pl.BlockSpec(memory_space=pl.ANY)
    out = pl.pallas_call(
        _kernel,
        in_specs=[any_spec] * 10,
        out_specs=pl.BlockSpec(memory_space=pltpu.VMEM),
        out_shape=jax.ShapeDtypeStruct((1, D), A_x.dtype),
        scratch_shapes=[
            pltpu.VMEM((1, D), BF16),
            pltpu.VMEM((1, D), BF16),
            pltpu.VMEM(w_mod.shape, BF16),
            pltpu.VMEM(A_wq.shape, BF16),
            pltpu.VMEM(wo.shape, BF16),
            pltpu.VMEM((3 * NG, 8, W + KPAD), BF16),
            pltpu.VMEM((2 * NG, 8, W), BF16),
            pltpu.VMEM(B_w_gate.shape, BF16),
            pltpu.VMEM(B_w_up.shape, BF16),
            pltpu.VMEM(B_w_down.shape, BF16),
            pltpu.VMEM((NH * DH, 128), F32),
            pltpu.VMEM((8, W), F32),
            pltpu.VMEM((NG, 8, 128), F32),
            pltpu.VMEM((6, 1, D), F32),
            pltpu.VMEM((8, D), F32),
            pltpu.SemaphoreType.DMA,
        ],
        compiler_params=pltpu.CompilerParams(vmem_limit_bytes=100 * 1024 * 1024),
    )(A_x.reshape(1, D), c, w_mod, A_wq, wo, kt, vt, B_w_gate, B_w_up, B_w_down)
    return out.reshape(B, Sq, D)
```
